```python
import jax
import jax.numpy as jnp

def _softmax(x, axis=-1):
    return jax.nn.softmax(x, axis=axis)

def _gelu(x):
    return jax.nn.gelu(x, approximate=True)

def _silu(x):
    return jax.nn.silu(x)

def _sigmoid(x):
    return jax.nn.sigmoid(x)

def _layernorm(x, axis=-1, eps=1e-05):
    m = jnp.mean(x, axis=axis, keepdims=True)
    v = jnp.var(x, axis=axis, keepdims=True)
    return (x - m) / jnp.sqrt(v + eps)

def _scatter_add(tgt, idx, src, axis=0):
    return tgt.at[idx].add(src)

def _segment_sum(src, seg, n):
    return jax.ops.segment_sum(src, seg, n)

class _Rng:

    def __init__(self, key):
        self._k = key

    def _next(self):
        self._k, sub = jax.random.split(self._k)
        return sub

    def normal(self, shape):
        return jax.random.normal(self._next(), shape, dtype=jnp.bfloat16)

    def randint(self, lo, hi, shape):
        return jax.random.randint(self._next(), shape, lo, hi, dtype=jnp.int32)

    def uniform(self, shape, lo=0.0, hi=1.0):
        return jax.random.uniform(self._next(), shape, jnp.bfloat16, lo, hi)

    def permutation(self, n):
        return jax.random.permutation(self._next(), n)
kernel_name = 'sequential_preLN__memory_aug_infini_attn__moe_arch_mod__prompt'

def setup_inputs():
    _rng = _Rng(jax.random.key(int.from_bytes(__import__("os").urandom(4), "little")))
    _w = lambda a: (lambda t: t.astype(jnp.bfloat16) if jnp.issubdtype(t.dtype, jnp.floating) else t)(jnp.asarray(a))

    def _A_setup():
        B, S, D, H = (1, 2048, 576, 32)
        N = 4
        L = max(1, S // N)
        sc = D ** (-0.5)
        return {'x': _w((lambda *s: _rng.normal(s) * 0.05)(B, N * L, D)), 'wq': _w((lambda *s: _rng.normal(s) * 0.05)(D, D) * sc), 'wk': _w((lambda *s: _rng.normal(s) * 0.05)(D, D) * sc), 'wv': _w((lambda *s: _rng.normal(s) * 0.05)(D, D) * sc), 'wo': _w((lambda *s: _rng.normal(s) * 0.05)(D, D) * sc), 'beta': _w((lambda *s: _rng.normal(s) * 0.05)(H))}
    _A_in = _A_setup()

    def _B_setup():
        B, S, D, F, C = (1, 2048, 576, 4608, 1)
        return {'x': _w((lambda *s: _rng.normal(s) * 0.05)(B, S, D)), 'w_r': _w((lambda *s: _rng.normal(s) * 0.05)(D)), 'w_gate': _w((lambda *s: _rng.normal(s) * 0.05)(D, F)), 'w_up': _w((lambda *s: _rng.normal(s) * 0.05)(D, F)), 'w_down': _w((lambda *s: _rng.normal(s) * 0.05)(F, D))}
    _B_in = _B_setup()
    return {'A_x': _A_in['x'], 'A_wq': _A_in['wq'], 'A_wk': _A_in['wk'], 'A_wv': _A_in['wv'], 'A_wo': _A_in['wo'], 'A_beta': _A_in['beta'], 'B_x': _B_in['x'], 'B_w_r': _B_in['w_r'], 'B_w_gate': _B_in['w_gate'], 'B_w_up': _B_in['w_up'], 'B_w_down': _B_in['w_down']}

def reference(A_x, A_wq, A_wk, A_wv, A_wo, A_beta, B_x, B_w_r, B_w_gate, B_w_up, B_w_down):

    def _A_ref(x, wq, wk, wv, wo, beta):
        B, S, D = x.shape
        H = 32
        Dh = D // H
        N = 4
        L = S // N
        q = (lambda x, *d: x.transpose(*d))((x @ wq).reshape(B, S, H, Dh), 0, 2, 1, 3).reshape(B, H, N, L, Dh)
        k = (lambda x, *d: x.transpose(*d))((x @ wk).reshape(B, S, H, Dh), 0, 2, 1, 3).reshape(B, H, N, L, Dh)
        v = (lambda x, *d: x.transpose(*d))((x @ wv).reshape(B, S, H, Dh), 0, 2, 1, 3).reshape(B, H, N, L, Dh)
        phi = lambda t: jnp.where(t > 0, t + 1.0, jnp.exp(t))
        scale = Dh ** (-0.5)
        ar = jnp.arange(L)
        mask = (lambda x, dt: x.astype(dt))(ar[:, None] < ar[None, :], x.dtype) * -1000000000.0
        g = _sigmoid(beta).reshape(1, H, 1, 1)
        M = jnp.einsum('bhd,bhe->bhde', q[:, :, 0, 0, :] * 0.0, q[:, :, 0, 0, :] * 0.0)
        z = q[:, :, 0, 0, :] * 0.0
        outs = []
        for s in range(N):
            qs, ks, vs = (q[:, :, s].copy(), k[:, :, s].copy(), v[:, :, s].copy())
            logits = jnp.einsum('bhqd,bhkd->bhqk', qs, ks) * scale + mask
            p = _softmax(logits, axis=-1)
            a_dot = jnp.einsum('bhqk,bhkd->bhqd', p, vs)
            pq = phi(qs)
            num = jnp.einsum('bhld,bhde->bhle', pq, M)
            den = jnp.einsum('bhld,bhd->bhl', pq, z)[..., None] + 1e-06
            a_mem = num / den
            o = g * a_mem + (1.0 - g) * a_dot
            outs.append(o)
            pk = phi(ks)
            M = M + jnp.einsum('bhld,bhle->bhde', pk, vs)
            z = z + jnp.einsum('bhld->bhd', pk)
        o = (lambda x, *d: x.transpose(*d))(jnp.stack(outs, 2).reshape(B, H, S, Dh), 0, 2, 1, 3).reshape(B, S, D)
        return o @ wo

    def _B_ref(x, w_r, w_gate, w_up, w_down):
        B, S, D = x.shape
        C = 1
        r = x @ w_r
        idx = jnp.argsort(-r, axis=-1)[:, :C]
        idx_e = jnp.repeat(idx.reshape(B, C, 1), D, axis=2)
        x_sel = jnp.take_along_axis(x, idx_e, axis=1)
        g = _silu(x_sel @ w_gate)
        u = x_sel @ w_up
        y = g * u @ w_down
        r_sel = _sigmoid(jnp.take_along_axis(r, idx, axis=1))
        y = y * r_sel.reshape(B, C, 1)
        b_off = (jnp.arange(B) * S).reshape(B, 1)
        flat_idx = (idx + b_off).reshape(B * C)
        zero = (x * 0.0).reshape(B * S, D)
        upd = _scatter_add(zero, flat_idx, y.reshape(B * C, D), axis=0)
        return x + upd.reshape(B, S, D)
    x = A_x
    h = x + _A_ref(_layernorm(x, axis=-1), A_wq, A_wk, A_wv, A_wo, A_beta)
    h2 = h + _B_ref(_layernorm(h, axis=-1), B_w_r, B_w_gate, B_w_up, B_w_down)
    return h2
```

```python
import numpy as np
import jax
import jax.numpy as jnp
from jax import lax
import jax.experimental.pallas as pl
import jax.experimental.pallas.tpu as pltpu

S, D, H, DH = 2048, 576, 32, 18
NSEG, L = 4, 512
F = 4608
HPT = 7
NT = 5
DP = NT * 128
LOG2E = float(np.log2(np.e))
QSCALE = float(DH ** -0.5) * LOG2E
EPS_BF16 = float(np.asarray(1e-5, dtype=jnp.bfloat16).astype(np.float32))

bf16 = jnp.bfloat16
f32 = jnp.float32
NT_DIMS = (((1,), (1,)), ((), ()))


def _rb(x):
    return x.astype(bf16).astype(f32)


def _layernorm_t(xf):
    m = jnp.mean(xf, axis=0, keepdims=True)
    c = xf - m
    v = jnp.mean(c * c, axis=0, keepdims=True)
    sd = _rb(jnp.sqrt(_rb(_rb(v) + EPS_BF16)))
    return (xf - _rb(m)) * (1.0 / sd)


def _pad_cols(w):
    lane = lax.broadcasted_iota(jnp.int32, (D, 128), 1)
    tiles = []
    for t in range(NT):
        lo = HPT * DH * t
        if t < NT - 1:
            tiles.append(jnp.where(lane < HPT * DH, w[:, lo:lo + 128], jnp.zeros((), w.dtype)))
        else:
            tiles.append(jnp.concatenate(
                [w[:, lo:], jnp.zeros((D, 128 - (D - lo)), w.dtype)], axis=1))
    return tiles


def _phi(t):
    return jnp.where(t > 0, t + 1.0, jnp.exp(t))


def _kernel(xt_hbm, wq_hbm, wk_hbm, wv_hbm, wo_hbm, beta_ref, wr_ref, wg_hbm, wu_hbm, wdt_hbm,
            o_hbm,
            xt_s, wq_s, wk_s, wv_s, wo_s, wqk_s, wvt_s, wot_s, g_s,
            lnt_s, q_s, k_s, pq_s, pk_s, vt_s, ot_s, ob_s, m_s, h_s, hn_s, r_s, out_s, patch_s,
            wg_s, wu_s, wdt_s, sem_x, sem_w, sem_f, sem_o):
    x_cp = [pltpu.make_async_copy(xt_hbm.at[:, s * L:(s + 1) * L], xt_s.at[s], sem_x.at[s])
            for s in range(NSEG)]
    w_cp = [pltpu.make_async_copy(src, dst, sem_w.at[i]) for i, (src, dst) in enumerate(
        [(wq_hbm, wq_s), (wk_hbm, wk_s), (wv_hbm, wv_s), (wo_hbm, wo_s)])]
    f_cp = [pltpu.make_async_copy(src, dst, sem_f.at[i]) for i, (src, dst) in enumerate(
        [(wg_hbm, wg_s), (wu_hbm, wu_s), (wdt_hbm, wdt_s)])]
    w_cp[0].start()
    w_cp[1].start()
    x_cp[0].start()
    w_cp[2].start()
    w_cp[3].start()
    for s in range(1, NSEG):
        x_cp[s].start()

    w_cp[0].wait()
    for t, tile in enumerate(_pad_cols(wq_s[...])):
        wqk_s[:, 128 * t:128 * (t + 1)] = tile
    w_cp[1].wait()
    for t, tile in enumerate(_pad_cols(wk_s[...])):
        wqk_s[:, DP + 128 * t:DP + 128 * (t + 1)] = tile
    w_cp[2].wait()
    for t, tile in enumerate(_pad_cols(wv_s[...])):
        wvt_s[128 * t:128 * (t + 1), :] = tile.T
    w_cp[3].wait()
    for t, tile in enumerate(_pad_cols(wo_s[...].T)):
        wot_s[:, 128 * t:128 * (t + 1)] = tile
    for c in f_cp:
        c.start()

    frow = lax.broadcasted_iota(jnp.int32, (DP, H), 0)
    hid = lax.broadcasted_iota(jnp.int32, (DP, H), 1)
    expand = ((frow % 128) // DH + (frow // 128) * HPT == hid) & (frow % 128 < HPT * DH)
    beta_b = jnp.broadcast_to(beta_ref[...].reshape(1, H), (128, H))
    beta_rows = lax.dot_general(expand.astype(bf16), beta_b, NT_DIMS, preferred_element_type=f32)
    g_s[...] = _rb(jax.nn.sigmoid(beta_rows))
    m_s[...] = jnp.zeros(m_s.shape, f32)

    def one_head(t, r):
        lane = lax.broadcasted_iota(jnp.int32, (128, 128), 1)
        krow = lax.broadcasted_iota(jnp.int32, (128, 128), 0)
        hm = (lane >= DH * r) & (lane < DH * (r + 1))
        causal = krow <= lane
        base = pl.multiple_of(128 * t + 16 * r, 16)
        for j in range(4):
            n = 128 * (j + 1)
            qj = jnp.where(hm, q_s[t, 128 * j:128 * (j + 1), :], jnp.zeros((), bf16))
            st = lax.dot_general(k_s[t, 0:n, :], qj, NT_DIMS, preferred_element_type=f32)
            diag = jnp.where(causal, st[n - 128:], -1e30)
            st = jnp.concatenate([st[:n - 128], diag], axis=0) if j > 0 else diag
            mx = jnp.max(st, axis=0, keepdims=True)
            p = jnp.exp2(st - mx)
            lsum = jnp.sum(p, axis=0, keepdims=True)
            acc = jnp.dot(vt_s[pl.ds(base, 32), 0:n], p.astype(bf16),
                          preferred_element_type=f32)
            acc = acc * (1.0 / lsum)
            cs = slice(128 * j, 128 * (j + 1))
            if r == 0:
                ot_s[pl.ds(base, 32), cs] = acc
            else:
                prev = ot_s[pl.ds(base, 16), cs]
                rowi = lax.broadcasted_iota(jnp.int32, (16, 128), 0)
                ot_s[pl.ds(base, 16), cs] = jnp.where(rowi >= 2 * r, acc[0:16], prev)
                ot_s[pl.ds(base + 16, 16), cs] = acc[16:32]

    def segment(s, carry):
        pltpu.make_async_copy(xt_s.at[s], xt_s.at[s], sem_x.at[s]).wait()
        xs = xt_s[s].astype(f32)
        lnt = _layernorm_t(xs).astype(bf16)
        lnt_s[...] = lnt
        ln = lnt.T
        qk = jnp.dot(ln, wqk_s[...], preferred_element_type=f32)
        for t in range(NT):
            qf = qk[:, 128 * t:128 * (t + 1)]
            kf = qk[:, DP + 128 * t:DP + 128 * (t + 1)]
            q_s[t] = (qf * QSCALE).astype(bf16)
            k_s[t] = kf.astype(bf16)
            pq_s[t] = _phi(_rb(qf)).astype(bf16)
            pk_s[t] = _phi(_rb(kf)).astype(bf16)
        vt_s[...] = jnp.dot(wvt_s[...], lnt, preferred_element_type=f32).astype(bf16)

        def tile_body(t, c):
            for r in range(HPT):
                one_head(t, r)
            return c
        lax.fori_loop(0, NT - 1, tile_body, 0)
        ot_s[128 * (NT - 1):, :] = jnp.zeros((128, L), f32)
        for r in range(H - HPT * (NT - 1)):
            one_head(NT - 1, r)

        @pl.when(s == 0)
        def _():
            for t in range(NT):
                g = g_s[128 * t:128 * (t + 1), :]
                g1 = _rb(1.0 - g)
                for j in range(4):
                    cs = slice(128 * j, 128 * (j + 1))
                    ob_s[128 * t:128 * (t + 1), cs] = (
                        g1 * ot_s[128 * t:128 * (t + 1), cs]).astype(bf16)

        @pl.when(s > 0)
        def _():
            erow = lax.broadcasted_iota(jnp.int32, (128, 128), 0)
            dcol = lax.broadcasted_iota(jnp.int32, (128, 128), 1)
            bd_mask = (erow // DH == dcol // DH) & (dcol < HPT * DH)
            for t in range(NT):
                mt = m_s[t]
                mb = jnp.where(bd_mask, mt, 0.0)
                zb = jnp.where(bd_mask, jnp.broadcast_to(mt[126:127, :], (128, 128)), 0.0)
                nd = lax.dot_general(jnp.concatenate([mb, zb], axis=0).astype(bf16), pq_s[t],
                                     NT_DIMS, preferred_element_type=f32)
                amem = nd[:128] / (nd[128:] + 1e-6)
                g = g_s[128 * t:128 * (t + 1), :]
                g1 = _rb(1.0 - g)
                for j in range(4):
                    cs = slice(128 * j, 128 * (j + 1))
                    ob_s[128 * t:128 * (t + 1), cs] = (
                        g * amem[:, cs] + g1 * ot_s[128 * t:128 * (t + 1), cs]).astype(bf16)

        attn = jnp.dot(wot_s[...], ob_s[...], preferred_element_type=f32)
        h = _rb(xs + _rb(attn))
        hn = _layernorm_t(h).astype(bf16)
        out_s[s] = (h + hn.astype(f32)).astype(bf16)
        pltpu.make_async_copy(out_s.at[s], o_hbm.at[:, pl.ds(pl.multiple_of(s * L, L), L)],
                              sem_o.at[s]).start()
        hb = h.astype(bf16)
        for j in range(4):
            h_s[4 * s + j] = hb[:, 128 * j:128 * (j + 1)]
            hn_s[4 * s + j] = hn[:, 128 * j:128 * (j + 1)]
        rr = jnp.dot(jnp.broadcast_to(wr_ref[...].reshape(1, D), (16, D)), hn,
                     preferred_element_type=f32)
        r_s[s] = rr[0:8]

        @pl.when(s < NSEG - 1)
        def _():
            for t in range(NT):
                vt = vt_s[128 * t:128 * (t + 1), :]
                rowl = lax.broadcasted_iota(jnp.int32, (128, L), 0)
                vt = jnp.where(rowl == 126, jnp.ones((), bf16), vt)
                m_s[t] = m_s[t] + jnp.dot(vt, pk_s[t], preferred_element_type=f32)
        return carry

    lax.fori_loop(0, NSEG, segment, 0)

    rall = jnp.concatenate([_rb(r_s[s][0:1]) for s in range(NSEG)], axis=0)
    rmax = jnp.max(rall)
    pos = (lax.broadcasted_iota(jnp.int32, (NSEG, L), 0) * L
           + lax.broadcasted_iota(jnp.int32, (NSEG, L), 1))
    idx = jnp.clip(jnp.min(jnp.where(rall == rmax, pos, S)), 0, S - 1)
    tt = idx // 128
    ln_sel = idx - tt * 128
    rsel = _rb(jax.nn.sigmoid(jnp.full((1, 1), rmax, f32)))
    hn_t = hn_s[tt]
    h_t = h_s[tt].astype(f32)
    onehot = (lax.broadcasted_iota(jnp.int32, (16, 128), 1) == ln_sel).astype(bf16)
    xsel = lax.dot_general(onehot, hn_t, NT_DIMS, preferred_element_type=f32).astype(bf16)

    f_cp[0].wait()
    f_cp[1].wait()
    gate = _rb(jnp.dot(xsel, wg_s[...], preferred_element_type=f32))
    up = _rb(jnp.dot(xsel, wu_s[...], preferred_element_type=f32))
    gu = (_rb(gate * jax.nn.sigmoid(gate)) * up).astype(bf16)
    f_cp[2].wait()
    y = _rb(lax.dot_general(gu, wdt_s[...], NT_DIMS, preferred_element_type=f32))
    y = _rb(y * rsel)
    yt = jnp.broadcast_to(y[0:1], (128, D)).T
    upd = jnp.where(lax.broadcasted_iota(jnp.int32, (D, 128), 1) == ln_sel, yt, 0.0)
    patch_s[...] = (h_t + _rb(hn_t.astype(f32) + upd)).astype(bf16)
    for s in range(NSEG):
        pltpu.make_async_copy(out_s.at[s], o_hbm.at[:, s * L:(s + 1) * L], sem_o.at[s]).wait()
    cp = pltpu.make_async_copy(patch_s, o_hbm.at[:, pl.ds(pl.multiple_of(tt * 128, 128), 128)],
                               sem_o.at[NSEG])
    cp.start()
    cp.wait()


@jax.jit
def pallas_sequential_preLN__memory_aug_infini_attn__moe_arch_mod__prompt_kernel(
    A_x: jax.Array,
    A_wq: jax.Array,
    A_wk: jax.Array,
    A_wv: jax.Array,
    A_wo: jax.Array,
    A_beta: jax.Array,
    B_x: jax.Array,
    B_w_r: jax.Array,
    B_w_gate: jax.Array,
    B_w_up: jax.Array,
    B_w_down: jax.Array,
):
    del B_x
    vmem = pl.BlockSpec(memory_space=pltpu.VMEM)
    hbm = pl.BlockSpec(memory_space=pltpu.HBM)
    out_t = pl.pallas_call(
        _kernel,
        out_shape=jax.ShapeDtypeStruct((D, S), bf16),
        in_specs=[hbm, hbm, hbm, hbm, hbm, vmem, vmem, hbm, hbm, hbm],
        out_specs=hbm,
        scratch_shapes=[
            pltpu.VMEM((NSEG, D, L), bf16),
            pltpu.VMEM((D, D), bf16),
            pltpu.VMEM((D, D), bf16),
            pltpu.VMEM((D, D), bf16),
            pltpu.VMEM((D, D), bf16),
            pltpu.VMEM((D, 2 * DP), bf16),
            pltpu.VMEM((DP, D), bf16),
            pltpu.VMEM((D, DP), bf16),
            pltpu.VMEM((DP, 128), f32),
            pltpu.VMEM((D, L), bf16),
            pltpu.VMEM((NT, L, 128), bf16),
            pltpu.VMEM((NT, L, 128), bf16),
            pltpu.VMEM((NT, L, 128), bf16),
            pltpu.VMEM((NT, L, 128), bf16),
            pltpu.VMEM((DP, L), bf16),
            pltpu.VMEM((DP, L), f32),
            pltpu.VMEM((DP, L), bf16),
            pltpu.VMEM((NT, 128, 128), f32),
            pltpu.VMEM((S // 128, D, 128), bf16),
            pltpu.VMEM((S // 128, D, 128), bf16),
            pltpu.VMEM((NSEG, 8, L), f32),
            pltpu.VMEM((NSEG, D, L), bf16),
            pltpu.VMEM((D, 128), bf16),
            pltpu.VMEM((D, F), bf16),
            pltpu.VMEM((D, F), bf16),
            pltpu.VMEM((D, F), bf16),
            pltpu.SemaphoreType.DMA((NSEG,)),
            pltpu.SemaphoreType.DMA((4,)),
            pltpu.SemaphoreType.DMA((3,)),
            pltpu.SemaphoreType.DMA((NSEG + 1,)),
        ],
        compiler_params=pltpu.CompilerParams(vmem_limit_bytes=100 * 1024 * 1024),
    )(A_x.reshape(S, D).T, A_wq, A_wk, A_wv, A_wo, A_beta, B_w_r,
      B_w_gate, B_w_up, B_w_down.T)
    return out_t.T.reshape(1, S, D)
```

```python
import numpy as np
import jax
import jax.numpy as jnp
from jax import lax
import jax.experimental.pallas as pl
import jax.experimental.pallas.tpu as pltpu

S, D, H, DH = 2048, 576, 32, 18
NSEG, L = 4, 512
F = 4608
HPT = 7
NT = 5
DP = NT * 128
LOG2E = float(np.log2(np.e))
QSCALE = float(DH ** -0.5) * LOG2E
EPS_BF16 = float(np.asarray(1e-5, dtype=jnp.bfloat16).astype(np.float32))

bf16 = jnp.bfloat16
f32 = jnp.float32
u32 = jnp.uint32
G = 4
LAG = 5
STEPS = [(j, i) for j in range(4) for i in range(j + 1)]
NT_DIMS = (((1,), (1,)), ((), ()))


def _rb(x):
    return x.astype(bf16).astype(f32)


def _layernorm_t(xf):
    m = jnp.mean(xf, axis=0, keepdims=True)
    c = xf - m
    v = jnp.mean(c * c, axis=0, keepdims=True)
    sd = _rb(jnp.sqrt(_rb(_rb(v) + EPS_BF16)))
    return (xf - _rb(m)) * (1.0 / sd)


def _pack(x):
    return pltpu.bitcast(x, u32)


def _unpack(x):
    return pltpu.bitcast(x, bf16)


def _pad_cols(w):
    w = _pack(w)
    rows = D // 2
    lane = lax.broadcasted_iota(jnp.int32, (rows, 128), 1)
    src = [w[:, 128 * i:128 * (i + 1)] for i in range(D // 128)]
    src.append(jnp.concatenate([w[:, 128 * (D // 128):], jnp.zeros((rows, 64), u32)], axis=1))
    tiles = []
    for t in range(NT):
        if t == 0:
            tile = src[0]
        else:
            tile = jnp.where(lane < 2 * t, pltpu.roll(src[t - 1], 2 * t, 1),
                             pltpu.roll(src[t], 2 * t, 1))
        valid = min(HPT * DH, D - HPT * DH * t)
        tiles.append(jnp.where(lane < valid, tile, jnp.uint32(0)))
    return tiles


def _phi(t):
    return jnp.where(t > 0, t + 1.0, jnp.exp(t))


def _kernel(xt_hbm, wq_hbm, wk_hbm, wv_hbm, wo_hbm, beta_ref, wr_ref, wg_hbm, wu_hbm, wdt_hbm,
            o_hbm,
            xt_s, wq_s, wk_s, wv_s, wo_s, wqk_s, wvt_s, wot_s, g_s,
            lnt_s, q_s, k_s, pq_s, pk_s, vt_s, ow_s, s0_s, s1_s, s2_s, s3_s, mx_s, acc_s, ob_s, m_s, h_s, hn_s, r_s, out_s, patch_s,
            wg_s, wu_s, wdt_s, sem_x, sem_w, sem_f, sem_o):
    x_cp = [pltpu.make_async_copy(xt_hbm.at[:, s * L:(s + 1) * L], xt_s.at[s], sem_x.at[s])
            for s in range(NSEG)]
    w_cp = [pltpu.make_async_copy(src, dst, sem_w.at[i]) for i, (src, dst) in enumerate(
        [(wq_hbm, wq_s), (wk_hbm, wk_s), (wv_hbm, wv_s), (wo_hbm, wo_s)])]
    f_cp = [pltpu.make_async_copy(src, dst, sem_f.at[i]) for i, (src, dst) in enumerate(
        [(wg_hbm, wg_s), (wu_hbm, wu_s), (wdt_hbm, wdt_s)])]
    w_cp[0].start()
    w_cp[1].start()
    x_cp[0].start()
    w_cp[2].start()
    w_cp[3].start()
    for s in range(1, NSEG):
        x_cp[s].start()

    w_cp[0].wait()
    for t, tile in enumerate(_pad_cols(wq_s[...])):
        wqk_s[:, 256 * t:256 * t + 128] = _unpack(tile)
    w_cp[1].wait()
    for t, tile in enumerate(_pad_cols(wk_s[...])):
        wqk_s[:, 256 * t + 128:256 * (t + 1)] = _unpack(tile)
    w_cp[2].wait()
    for t, tile in enumerate(_pad_cols(wv_s[...])):
        wvt_s[128 * t:128 * (t + 1), :] = _unpack(tile).T
    w_cp[3].wait()
    for t, tile in enumerate(_pad_cols(wo_s[...].T)):
        wot_s[:, 128 * t:128 * (t + 1)] = _unpack(tile)
    for c in f_cp:
        c.start()

    frow = lax.broadcasted_iota(jnp.int32, (DP, H), 0)
    hid = lax.broadcasted_iota(jnp.int32, (DP, H), 1)
    expand = ((frow % 128) // DH + (frow // 128) * HPT == hid) & (frow % 128 < HPT * DH)
    beta_b = jnp.broadcast_to(beta_ref[...].reshape(1, H), (128, H))
    beta_rows = lax.dot_general(expand.astype(bf16), beta_b, NT_DIMS, preferred_element_type=f32)
    g_s[...] = _rb(jax.nn.sigmoid(beta_rows))
    m_s[...] = jnp.zeros(m_s.shape, f32)
    for ref in (s2_s, s3_s, mx_s):
        ref[...] = jnp.zeros(ref.shape, f32)
    acc_s[...] = jnp.ones(acc_s.shape, f32)

    def head_info(h):
        t = h // HPT
        r = h - HPT * t
        return t, r, pl.multiple_of(64 * t + 8 * r, 8)

    s_refs = [s0_s, s1_s, s2_s, s3_s]

    def qk_step(heads, j, i, qs, mx):
        for a, (h, t, r, base) in enumerate(heads):
            kk = _unpack(k_s[t, 64 * i:64 * (i + 1), :])
            st = lax.dot_general(kk, qs[a], NT_DIMS, preferred_element_type=f32)
            if i == j:
                krow = lax.broadcasted_iota(jnp.int32, (128, 128), 0)
                qcol = lax.broadcasted_iota(jnp.int32, (128, 128), 1)
                st = jnp.where(krow <= qcol, st, -1e30)
            s_refs[j][a, 128 * i:128 * (i + 1), :] = st
            m8 = jnp.max(st.reshape(16, 8, 128), axis=0)
            mx[a] = m8 if i == 0 else jnp.maximum(mx[a], m8)
            if i == j:
                mx_s[j, a] = jnp.broadcast_to(jnp.max(mx[a], axis=0, keepdims=True), (8, 128))

    def sm_step(heads, j, i, acc, load_acc, store_acc):
        for a, (h, t, r, base) in enumerate(heads):
            st = s_refs[j][a, 128 * i:128 * (i + 1), :]
            m = mx_s[j, a]
            p = jnp.exp2(st.reshape(16, 8, 128) - m[None]).reshape(128, 128).astype(bf16)
            vw = vt_s[pl.ds(base, 16), 128 * i:128 * (i + 1)]
            vw = jnp.where(lax.broadcasted_iota(jnp.int32, (16, 128), 0) == 15,
                           jnp.uint32(0x3F803F80), vw)
            d = jnp.dot(_unpack(vw), p, preferred_element_type=f32)
            if load_acc:
                acc[a] = acc_s[a] + d
            else:
                acc[a] = d if i == 0 else acc[a] + d
            if i == j:
                ow_s[h + G, :, 128 * j:128 * (j + 1)] = acc[a] * (1.0 / acc[a][30:31])
            elif store_acc:
                acc_s[a] = acc[a]

    def sm_tail(heads):
        acc = [None] * G
        for n in range(10 - LAG, 10):
            j, i = STEPS[n]
            sm_step(heads, j, i, acc, load_acc=(n == 10 - LAG and i > 0), store_acc=False)
            yield

    def group_body(g, carry):
        cur, prev, qmask = [], [], []
        lane64 = lax.broadcasted_iota(jnp.int32, (64, 128), 1)
        for a in range(G):
            h = G * g + a
            t, r, base = head_info(h)
            cur.append((h, t, r, base))
            qmask.append((lane64 >= DH * r) & (lane64 < DH * (r + 1)))
            prev.append((h - G,) + head_info(jnp.maximum(h - G, 0)))
        tail = sm_tail(prev)
        acc = [None] * G
        qs, mx = None, [None] * G
        for n in range(10):
            j, i = STEPS[n]
            if i == 0:
                qs = [_unpack(jnp.where(qmask[a], q_s[cur[a][1], 64 * j:64 * (j + 1), :],
                                        jnp.uint32(0))) for a in range(G)]
            qk_step(cur, j, i, qs, mx)
            if n < LAG:
                next(tail)
            else:
                jj, ii = STEPS[n - LAG]
                sm_step(cur, jj, ii, acc, load_acc=False, store_acc=(n == 9))
        return carry

    def segment(s, carry):
        pltpu.make_async_copy(xt_s.at[s], xt_s.at[s], sem_x.at[s]).wait()
        xs = xt_s[s].astype(f32)
        lnt = _layernorm_t(xs).astype(bf16)
        lnt_s[...] = lnt
        ln = lnt.T
        for t in range(NT):
            qk = jnp.dot(ln, wqk_s[:, 256 * t:256 * (t + 1)], preferred_element_type=f32)
            qf, kf = qk[:, :128], qk[:, 128:]
            q_s[t] = _pack((qf * QSCALE).astype(bf16))
            k_s[t] = _pack(kf.astype(bf16))
            pq_s[t] = _pack(_phi(qf).astype(bf16))
            pk_s[t] = _pack(_phi(kf).astype(bf16))
        for t in range(NT):
            vt = jnp.dot(wvt_s[128 * t:128 * (t + 1), :], lnt, preferred_element_type=f32)
            vt_s[64 * t:64 * (t + 1), :] = _pack(vt.astype(bf16))

        lax.fori_loop(0, H // G, group_body, 0, unroll=2)
        for _ in sm_tail([(h, h // HPT, h % HPT, 64 * (h // HPT) + 8 * (h % HPT))
                          for h in range(H - G, H)]):
            pass

        def dot_part(t, cs):
            rowi = lax.broadcasted_iota(jnp.int32, (16, 128), 0)
            parts = []
            for rr in range(8):
                h = HPT * t + rr
                lo = ow_s[h - 1 + G, 16:32, cs] if (rr > 0 and h - 1 < H) else None
                hi = ow_s[h + G, 0:16, cs] if (rr < HPT and h < H) else None
                if lo is None and hi is None:
                    parts.append(jnp.zeros((16, 128), f32))
                elif lo is None or hi is None:
                    parts.append(hi if lo is None else lo)
                else:
                    parts.append(jnp.where(rowi >= 2 * rr, hi, lo))
            return jnp.concatenate(parts, axis=0)

        @pl.when(s == 0)
        def _():
            for t in range(NT):
                g = g_s[128 * t:128 * (t + 1), :]
                g1 = _rb(1.0 - g)
                for j in range(4):
                    cs = slice(128 * j, 128 * (j + 1))
                    ob_s[128 * t:128 * (t + 1), cs] = (
                        g1 * dot_part(t, cs)).astype(bf16)

        @pl.when(s > 0)
        def _():
            erow = lax.broadcasted_iota(jnp.int32, (128, 128), 0)
            dcol = lax.broadcasted_iota(jnp.int32, (128, 128), 1)
            bd_mask = (erow // DH == dcol // DH) & (dcol < HPT * DH)
            for t in range(NT):
                mt = m_s[t]
                mb = jnp.where(bd_mask, mt, 0.0)
                zb = jnp.where(bd_mask, jnp.broadcast_to(mt[126:127, :], (128, 128)), 0.0)
                nd = lax.dot_general(jnp.concatenate([mb, zb], axis=0).astype(bf16), _unpack(pq_s[t]),
                                     NT_DIMS, preferred_element_type=f32)
                amem = nd[:128] / (nd[128:] + 1e-6)
                g = g_s[128 * t:128 * (t + 1), :]
                g1 = _rb(1.0 - g)
                for j in range(4):
                    cs = slice(128 * j, 128 * (j + 1))
                    ob_s[128 * t:128 * (t + 1), cs] = (
                        g * amem[:, cs] + g1 * dot_part(t, cs)).astype(bf16)

        attn = jnp.dot(wot_s[...], ob_s[...], preferred_element_type=f32)
        h = _rb(xs + _rb(attn))
        hn = _layernorm_t(h).astype(bf16)
        out_s[s] = (h + hn.astype(f32)).astype(bf16)
        pltpu.make_async_copy(out_s.at[s], o_hbm.at[:, pl.ds(pl.multiple_of(s * L, L), L)],
                              sem_o.at[s]).start()
        hb = h.astype(bf16)
        for j in range(4):
            h_s[4 * s + j] = hb[:, 128 * j:128 * (j + 1)]
            hn_s[4 * s + j] = hn[:, 128 * j:128 * (j + 1)]
        rr = jnp.dot(jnp.broadcast_to(wr_ref[...].reshape(1, D), (16, D)), hn,
                     preferred_element_type=f32)
        r_s[s] = rr[0:8]

        @pl.when(s < NSEG - 1)
        def _():
            for t in range(NT):
                vt = vt_s[64 * t:64 * (t + 1), :]
                rowl = lax.broadcasted_iota(jnp.int32, (64, L), 0)
                vt = _unpack(jnp.where(rowl == 63, jnp.uint32(0x3F803F80), vt))
                m_s[t] = m_s[t] + jnp.dot(vt, _unpack(pk_s[t]), preferred_element_type=f32)
        return carry

    lax.fori_loop(0, NSEG, segment, 0)

    rall = jnp.concatenate([_rb(r_s[s][0:1]) for s in range(NSEG)], axis=0)
    rmax = jnp.max(rall)
    pos = (lax.broadcasted_iota(jnp.int32, (NSEG, L), 0) * L
           + lax.broadcasted_iota(jnp.int32, (NSEG, L), 1))
    idx = jnp.clip(jnp.min(jnp.where(rall == rmax, pos, S)), 0, S - 1)
    tt = idx // 128
    ln_sel = idx - tt * 128
    rsel = _rb(jax.nn.sigmoid(jnp.full((1, 1), rmax, f32)))
    hn_t = hn_s[tt]
    h_t = h_s[tt].astype(f32)
    onehot = (lax.broadcasted_iota(jnp.int32, (16, 128), 1) == ln_sel).astype(bf16)
    xsel = lax.dot_general(onehot, hn_t, NT_DIMS, preferred_element_type=f32).astype(bf16)

    f_cp[0].wait()
    f_cp[1].wait()
    gate = _rb(jnp.dot(xsel, wg_s[...], preferred_element_type=f32))
    up = _rb(jnp.dot(xsel, wu_s[...], preferred_element_type=f32))
    gu = (_rb(gate * jax.nn.sigmoid(gate)) * up).astype(bf16)
    f_cp[2].wait()
    y = _rb(lax.dot_general(gu, wdt_s[...], NT_DIMS, preferred_element_type=f32))
    y = _rb(y * rsel)
    yt = jnp.broadcast_to(y[0:1], (128, D)).T
    upd = jnp.where(lax.broadcasted_iota(jnp.int32, (D, 128), 1) == ln_sel, yt, 0.0)
    patch_s[...] = (h_t + _rb(hn_t.astype(f32) + upd)).astype(bf16)
    for s in range(NSEG):
        pltpu.make_async_copy(out_s.at[s], o_hbm.at[:, s * L:(s + 1) * L], sem_o.at[s]).wait()
    cp = pltpu.make_async_copy(patch_s, o_hbm.at[:, pl.ds(pl.multiple_of(tt * 128, 128), 128)],
                               sem_o.at[NSEG])
    cp.start()
    cp.wait()


@jax.jit
def pallas_sequential_preLN__memory_aug_infini_attn__moe_arch_mod__prompt_kernel(
    A_x: jax.Array,
    A_wq: jax.Array,
    A_wk: jax.Array,
    A_wv: jax.Array,
    A_wo: jax.Array,
    A_beta: jax.Array,
    B_x: jax.Array,
    B_w_r: jax.Array,
    B_w_gate: jax.Array,
    B_w_up: jax.Array,
    B_w_down: jax.Array,
):
    del B_x
    vmem = pl.BlockSpec(memory_space=pltpu.VMEM)
    hbm = pl.BlockSpec(memory_space=pltpu.HBM)
    out_t = pl.pallas_call(
        _kernel,
        out_shape=jax.ShapeDtypeStruct((D, S), bf16),
        in_specs=[hbm, hbm, hbm, hbm, hbm, vmem, vmem, hbm, hbm, hbm],
        out_specs=hbm,
        scratch_shapes=[
            pltpu.VMEM((NSEG, D, L), bf16),
            pltpu.VMEM((D, D), bf16),
            pltpu.VMEM((D, D), bf16),
            pltpu.VMEM((D, D), bf16),
            pltpu.VMEM((D, D), bf16),
            pltpu.VMEM((D, 2 * DP), bf16),
            pltpu.VMEM((DP, D), bf16),
            pltpu.VMEM((D, DP), bf16),
            pltpu.VMEM((DP, 128), f32),
            pltpu.VMEM((D, L), bf16),
            pltpu.VMEM((NT, L // 2, 128), u32),
            pltpu.VMEM((NT, L // 2, 128), u32),
            pltpu.VMEM((NT, L // 2, 128), u32),
            pltpu.VMEM((NT, L // 2, 128), u32),
            pltpu.VMEM((DP // 2, L), u32),
            pltpu.VMEM((H + G, 32, L), f32),
            pltpu.VMEM((G, 128, 128), f32),
            pltpu.VMEM((G, 256, 128), f32),
            pltpu.VMEM((G, 384, 128), f32),
            pltpu.VMEM((G, 512, 128), f32),
            pltpu.VMEM((4, G, 8, 128), f32),
            pltpu.VMEM((G, 32, 128), f32),
            pltpu.VMEM((DP, L), bf16),
            pltpu.VMEM((NT, 128, 128), f32),
            pltpu.VMEM((S // 128, D, 128), bf16),
            pltpu.VMEM((S // 128, D, 128), bf16),
            pltpu.VMEM((NSEG, 8, L), f32),
            pltpu.VMEM((NSEG, D, L), bf16),
            pltpu.VMEM((D, 128), bf16),
            pltpu.VMEM((D, F), bf16),
            pltpu.VMEM((D, F), bf16),
            pltpu.VMEM((D, F), bf16),
            pltpu.SemaphoreType.DMA((NSEG,)),
            pltpu.SemaphoreType.DMA((4,)),
            pltpu.SemaphoreType.DMA((3,)),
            pltpu.SemaphoreType.DMA((NSEG + 1,)),
        ],
        compiler_params=pltpu.CompilerParams(vmem_limit_bytes=100 * 1024 * 1024),
    )(A_x.reshape(S, D).T, A_wq, A_wk, A_wv, A_wo, A_beta, B_w_r,
      B_w_gate, B_w_up, B_w_down.T)
    return out_t.T.reshape(1, S, D)
```

```python
import numpy as np
import jax
import jax.numpy as jnp
from jax import lax
import jax.experimental.pallas as pl
import jax.experimental.pallas.tpu as pltpu

S, D, H, DH = 2048, 576, 32, 18
NSEG, L = 4, 512
F = 4608
HPT = 7
NT = 5
DP = NT * 128
LOG2E = float(np.log2(np.e))
QSCALE = float(DH ** -0.5) * LOG2E
EPS_BF16 = float(np.asarray(1e-5, dtype=jnp.bfloat16).astype(np.float32))

bf16 = jnp.bfloat16
f32 = jnp.float32
u32 = jnp.uint32
G = 4
LAG = 5
STEPS = [(j, i) for j in range(4) for i in range(j + 1)]
NT_DIMS = (((1,), (1,)), ((), ()))


def _rb(x):
    return x.astype(bf16).astype(f32)


def _layernorm_t(xf):
    m = jnp.sum(xf, axis=0, keepdims=True) * (1.0 / D)
    c = xf - m
    v = jnp.sum(c * c, axis=0, keepdims=True) * (1.0 / D)
    sd = _rb(jnp.sqrt(_rb(_rb(v) + EPS_BF16)))
    return c * (1.0 / sd)


def _pack(x):
    return pltpu.bitcast(x, u32)


def _unpack(x):
    return pltpu.bitcast(x, bf16)


def _head_rows(w):
    row = lax.broadcasted_iota(jnp.int32, (64, w.shape[1]), 0)
    w = jnp.concatenate([w, jnp.zeros((64, w.shape[1]), u32)], axis=0)
    for t in range(NT):
        lo = HPT * DH * t // 2
        valid = min(HPT * DH, D - HPT * DH * t) // 2
        yield jnp.where(row < valid, w[lo:lo + 64], jnp.uint32(0))


def _transposed(w):
    cols = [w[:, 128 * i:128 * (i + 1)] for i in range(D // 128)]
    cols.append(jnp.concatenate([w[:, 128 * (D // 128):], jnp.zeros((D, 64), bf16)], axis=1))
    return jnp.concatenate([_pack(c.T) for c in cols], axis=0)[:D // 2]


def _interleave(*gens):
    gens = list(gens)
    while gens:
        for g in list(gens):
            try:
                next(g)
            except StopIteration:
                gens.remove(g)


def _phi(t):
    return jnp.where(t > 0, t + 1.0, jnp.exp(t))


def _kernel(xt_hbm, wq_hbm, wk_hbm, wv_hbm, wo_hbm, beta_ref, wr_ref, wg_hbm, wu_hbm, wdt_hbm,
            o_hbm,
            xt_s, wq_s, wk_s, wv_s, wo_s, wc_s, wot_s, gl_s, g1_s,
            lnt_s, q_s, k_s, vt_s, am_s, ow_s, s0_s, s1_s, s2_s, s3_s, mx_s, acc_s,
            m_s, h_s, hn_s, r_s, out_s, patch_s,
            wg_s, wu_s, wdt_s, sem_x, sem_w, sem_f, sem_o):
    x_cp = [pltpu.make_async_copy(xt_hbm.at[:, s * L:(s + 1) * L], xt_s.at[s], sem_x.at[s])
            for s in range(NSEG)]
    w_cp = [pltpu.make_async_copy(src, dst, sem_w.at[i]) for i, (src, dst) in enumerate(
        [(wq_hbm, wq_s), (wk_hbm, wk_s), (wv_hbm, wv_s), (wo_hbm, wo_s)])]
    f_cp = [pltpu.make_async_copy(src, dst, sem_f.at[i]) for i, (src, dst) in enumerate(
        [(wg_hbm, wg_s), (wu_hbm, wu_s), (wdt_hbm, wdt_s)])]
    w_cp[0].start()
    w_cp[1].start()
    x_cp[0].start()
    w_cp[2].start()
    w_cp[3].start()

    g = _rb(jax.nn.sigmoid(beta_ref[...].astype(f32).reshape(1, H)))
    hrow = lax.broadcasted_iota(jnp.int32, (H, DP), 0)
    fcol = lax.broadcasted_iota(jnp.int32, (H, DP), 1)
    expand = ((fcol % 128) // DH + (fcol // 128) * HPT == hrow) & (fcol % 128 < HPT * DH)
    gl_s[...] = jnp.dot(jnp.broadcast_to(g, (16, H)).astype(bf16), expand.astype(bf16),
                        preferred_element_type=f32)[0:8]
    pick = (lax.broadcasted_iota(jnp.int32, ((H + G) * 8, H), 0) // 8 - G
            == lax.broadcasted_iota(jnp.int32, ((H + G) * 8, H), 1))
    g1_s[...] = lax.dot_general(pick.astype(bf16),
                                jnp.broadcast_to(_rb(1.0 - g), (128, H)).astype(bf16), NT_DIMS,
                                preferred_element_type=f32).reshape(H + G, 8, 128)
    m_s[...] = jnp.zeros(m_s.shape, f32)
    for ref in (s2_s, s3_s, mx_s):
        ref[...] = jnp.zeros(ref.shape, f32)
    acc_s[...] = jnp.ones(acc_s.shape, f32)

    def ln_steps(load, store):
        xf = load()
        m = jnp.sum(xf, axis=0, keepdims=True) * (1.0 / D)
        yield
        c = xf - m
        v = jnp.sum(c * c, axis=0, keepdims=True) * (1.0 / D)
        yield
        sd = _rb(jnp.sqrt(_rb(_rb(v) + EPS_BF16)))
        store(xf, c * (1.0 / sd))
        yield

    def ln1_tile(s, j):
        def store(xf, y):
            lnt_s[:, 128 * j:128 * (j + 1)] = _pack(y.astype(bf16))
        return ln_steps(lambda: xt_s[s, :, 128 * j:128 * (j + 1)].astype(f32), store)

    def head_info(h):
        t = h // HPT
        r = h - HPT * t
        return t, r, pl.multiple_of(64 * t + 8 * r, 8)

    s_refs = [s0_s, s1_s, s2_s, s3_s]

    def qk_step(heads, j, i, qs, mx):
        for a, (h, t, r, base) in enumerate(heads):
            kk = _unpack(k_s[t, 64 * i:64 * (i + 1), :])
            st = jnp.dot(kk, qs[a], preferred_element_type=f32)
            if i == j:
                krow = lax.broadcasted_iota(jnp.int32, (128, 128), 0)
                qcol = lax.broadcasted_iota(jnp.int32, (128, 128), 1)
                st = jnp.where(krow <= qcol, st, -1e30)
            s_refs[j][a, 128 * i:128 * (i + 1), :] = st
            m8 = jnp.max(st.reshape(16, 8, 128), axis=0)
            mx[a] = m8 if i == 0 else jnp.maximum(mx[a], m8)
            if i == j:
                mx_s[j, a] = jnp.broadcast_to(jnp.max(mx[a], axis=0, keepdims=True), (8, 128))

    def sm_step(heads, j, i, acc, load_acc, store_acc):
        for a, (h, t, r, base) in enumerate(heads):
            st = s_refs[j][a, 128 * i:128 * (i + 1), :]
            m = mx_s[j, a]
            p = jnp.exp2(st.reshape(16, 8, 128) - m[None]).reshape(128, 128).astype(bf16)
            vw = vt_s[pl.ds(base, 16), 128 * i:128 * (i + 1)]
            vw = jnp.where(lax.broadcasted_iota(jnp.int32, (16, 128), 0) == 15,
                           jnp.uint32(0x3F803F80), vw)
            d = jnp.dot(_unpack(vw), p, preferred_element_type=f32)
            if load_acc:
                acc[a] = acc_s[a] + d
            else:
                acc[a] = d if i == 0 else acc[a] + d
            if i == j:
                scale = g1_s[h + G] / acc[a][24:32]
                ow_s[h + G, :, 128 * j:128 * (j + 1)] = acc[a] * scale[6:7]
            elif store_acc:
                acc_s[a] = acc[a]

    def sm_tail(heads):
        acc = [None] * G
        for n in range(10 - LAG, 10):
            j, i = STEPS[n]
            sm_step(heads, j, i, acc, load_acc=(n == 10 - LAG and i > 0), store_acc=False)
            yield

    def group_body(g, carry):
        cur, prev, qmask = [], [], []
        row64 = lax.broadcasted_iota(jnp.int32, (64, 128), 0)
        for a in range(G):
            h = G * g + a
            t, r, base = head_info(h)
            cur.append((h, t, r, base))
            qmask.append((row64 >= (DH // 2) * r) & (row64 < (DH // 2) * (r + 1)))
            prev.append((h - G,) + head_info(jnp.maximum(h - G, 0)))
        tail = sm_tail(prev)
        acc = [None] * G
        qs, mx = None, [None] * G
        for n in range(10):
            j, i = STEPS[n]
            if i == 0:
                qs = [_unpack(jnp.where(qmask[a], q_s[cur[a][1], :, 128 * j:128 * (j + 1)],
                                        jnp.uint32(0))) for a in range(G)]
            qk_step(cur, j, i, qs, mx)
            if n < LAG:
                next(tail)
            else:
                jj, ii = STEPS[n - LAG]
                sm_step(cur, jj, ii, acc, load_acc=False, store_acc=(n == 9))
        return carry

    def project(t):
        rows = 64 if t < NT - 1 else 40
        w = wc_s[t]
        w = jnp.concatenate([w[0:rows], w[64:64 + rows], w[128:128 + rows]], axis=0)
        qkv = jnp.dot(_unpack(w), _unpack(lnt_s[...]), preferred_element_type=f32)
        n = 2 * rows

        def full(x):
            return x if n == 128 else jnp.concatenate(
                [x, jnp.zeros((128 - n,) + x.shape[1:], x.dtype)], axis=0)

        qf, kf, vf = full(qkv[0:n]), full(qkv[n:2 * n]), full(qkv[2 * n:3 * n])
        q_s[t] = _pack((qf * QSCALE).astype(bf16))
        k_s[t] = _pack(kf.astype(bf16).T)
        vt = _pack(vf.astype(bf16))
        vt_s[64 * t:64 * (t + 1), :] = vt
        pq = _phi(qf).astype(bf16)
        pk = _phi(kf).astype(bf16)
        erow = lax.broadcasted_iota(jnp.int32, (128, 128), 0)
        dcol = lax.broadcasted_iota(jnp.int32, (128, 128), 1)
        bd_mask = (erow // DH == dcol // DH) & (dcol < HPT * DH)
        zrow = lax.broadcasted_iota(jnp.int32, (16, 128), 0)
        zcol = lax.broadcasted_iota(jnp.int32, (16, 128), 1)
        z_mask = (zcol // DH == zrow) & (zcol < HPT * DH)
        mt = m_s[t]
        mb = jnp.where(bd_mask, mt * gl_s[0:1, 128 * t:128 * (t + 1)], 0.0)
        zb = jnp.where(z_mask, jnp.broadcast_to(mt[126:127, :], (16, 128)), 0.0)
        nd = jnp.dot(jnp.concatenate([mb, zb], axis=0).astype(bf16), pq,
                     preferred_element_type=f32)
        inv = 1.0 / (nd[128:136] + 1e-6)
        row8 = lax.broadcasted_iota(jnp.int32, (8, L), 0)
        bro = [jnp.broadcast_to(inv[a:a + 1], (8, L)) for a in range(HPT)]
        for u in range(16):
            ha, hb = (8 * u) // DH, min((8 * u + 7) // DH, HPT - 1)
            sc = bro[ha] if ha == hb else jnp.where(row8 < DH * hb - 8 * u, bro[ha], bro[hb])
            am_s[128 * t + 8 * u:128 * t + 8 * (u + 1), :] = nd[8 * u:8 * (u + 1)] * sc
        vone = jnp.where(lax.broadcasted_iota(jnp.int32, (64, L), 0) == 63,
                         jnp.uint32(0x3F803F80), vt)
        m_s[t] = mt + lax.dot_general(_unpack(vone), pk, NT_DIMS, preferred_element_type=f32)

    def mix_tile(j, box):
        cs = slice(128 * j, 128 * (j + 1))
        row8 = lax.broadcasted_iota(jnp.int32, (8, 128), 0)
        parts = []
        for t in range(NT):
            for u in range(16):
                rr, half = u // 2, u % 2
                h = HPT * t + rr
                cut = 2 * rr - 8 * half
                lo_ok, hi_ok = (rr > 0 and h - 1 < H), (rr < HPT and h < H)
                lo = ow_s[h - 1 + G, 16 + 8 * half:24 + 8 * half, cs] if lo_ok else None
                hi = ow_s[h + G, 8 * half:8 * half + 8, cs] if hi_ok else None
                if cut <= 0 or not lo_ok:
                    dp = hi
                elif cut >= 8 or not hi_ok:
                    dp = lo
                else:
                    dp = jnp.where(row8 >= cut, hi, lo)
                am = am_s[128 * t + 8 * u:128 * t + 8 * (u + 1), cs]
                parts.append(am if dp is None else am + dp)
            if t % 2 == 1:
                yield
        box[j] = jnp.concatenate(parts, axis=0).astype(bf16)
        yield

    def out_proj_tile(s, j, ob, box):
        cs = slice(128 * j, 128 * (j + 1))
        chunks = []
        for c in range(4):
            w = _unpack(wot_s[72 * c:72 * (c + 1), :])
            attn = jnp.dot(w, ob, preferred_element_type=f32)
            chunks.append((xt_s[s, 144 * c:144 * (c + 1), cs].astype(f32) + attn).astype(bf16))
            yield
        box[j] = jnp.concatenate(chunks, axis=0)

    def ln2_tile(s, j, box):
        cs = slice(128 * j, 128 * (j + 1))

        def store(h, hn):
            hnb = hn.astype(bf16)
            out_s[s, :, cs] = (h + hn).astype(bf16)
            h_s[4 * s + j] = _pack(box[j])
            hn_s[4 * s + j] = _pack(hnb)
            rr = jnp.dot(jnp.broadcast_to(wr_ref[...].reshape(1, D), (16, D)), hnb,
                         preferred_element_type=f32)
            r_s[s, :, cs] = rr[0:8]
        return ln_steps(lambda: box[j].astype(f32), store)

    w_cp[0].wait()
    wqt = _transposed(wq_s[...])
    w_cp[1].wait()
    wkt = _transposed(wk_s[...])
    x_cp[0].wait()
    for s in range(1, NSEG):
        x_cp[s].start()
    _interleave(*[ln1_tile(0, j) for j in range(4)])
    w_cp[2].wait()
    wvt = _transposed(wv_s[...])
    w_cp[3].wait()
    for c in f_cp:
        c.start()
    for t, (tq, tk, tv, to) in enumerate(zip(_head_rows(wqt), _head_rows(wkt), _head_rows(wvt),
                                             _head_rows(_pack(wo_s[...])))):
        wc_s[t] = jnp.concatenate([tq, tk, tv], axis=0)
        project(t)
        wot_s[:, 128 * t:128 * (t + 1)] = _pack(_unpack(to).T)

    def segment(s, carry):
        @pl.when(s < NSEG - 1)
        def _():
            pltpu.make_async_copy(xt_s.at[s + 1], xt_s.at[s + 1], sem_x.at[s + 1]).wait()

        lax.fori_loop(0, H // G, group_body, 0, unroll=2)

        tail = sm_tail([(h, h // HPT, h % HPT, 64 * (h // HPT) + 8 * (h % HPT))
                        for h in range(H - G, H)])
        nxt = jnp.minimum(s + 1, NSEG - 1)
        obs, hs = {}, {}
        _interleave(mix_tile(0, obs), tail)
        for j in range(4):
            gens = [out_proj_tile(s, j, obs[j], hs), ln1_tile(nxt, j)]
            if j < 3:
                gens.append(mix_tile(j + 1, obs))
            if j > 0:
                gens.append(ln2_tile(s, j - 1, hs))
            _interleave(*gens)
        _interleave(ln2_tile(s, 3, hs))
        pltpu.make_async_copy(out_s.at[s], o_hbm.at[:, pl.ds(pl.multiple_of(s * L, L), L)],
                              sem_o.at[s]).start()

        @pl.when(s < NSEG - 1)
        def _():
            for t in range(NT):
                project(t)
        return carry

    lax.fori_loop(0, NSEG, segment, 0)

    rall = jnp.concatenate([_rb(r_s[s][0:1]) for s in range(NSEG)], axis=0)
    rmax = jnp.max(rall)
    pos = (lax.broadcasted_iota(jnp.int32, (NSEG, L), 0) * L
           + lax.broadcasted_iota(jnp.int32, (NSEG, L), 1))
    idx = jnp.clip(jnp.min(jnp.where(rall == rmax, pos, S)), 0, S - 1)
    tt = idx // 128
    ln_sel = idx - tt * 128
    rsel = _rb(jax.nn.sigmoid(jnp.full((1, 1), rmax, f32)))
    hn_t = _unpack(hn_s[tt])
    h_t = _unpack(h_s[tt]).astype(f32)
    onehot = (lax.broadcasted_iota(jnp.int32, (16, 128), 1) == ln_sel).astype(bf16)
    xsel = lax.dot_general(onehot, hn_t, NT_DIMS, preferred_element_type=f32).astype(bf16)

    f_cp[0].wait()
    f_cp[1].wait()
    gate = _rb(jnp.dot(xsel, wg_s[...], preferred_element_type=f32))
    up = _rb(jnp.dot(xsel, wu_s[...], preferred_element_type=f32))
    gu = (_rb(gate * jax.nn.sigmoid(gate)) * up).astype(bf16)
    f_cp[2].wait()
    y = _rb(lax.dot_general(gu, wdt_s[...], NT_DIMS, preferred_element_type=f32))
    y = _rb(y * rsel)
    yt = jnp.broadcast_to(y[0:1], (128, D)).T
    upd = jnp.where(lax.broadcasted_iota(jnp.int32, (D, 128), 1) == ln_sel, yt, 0.0)
    patch_s[...] = (h_t + _rb(hn_t.astype(f32) + upd)).astype(bf16)
    for s in range(NSEG):
        pltpu.make_async_copy(out_s.at[s], o_hbm.at[:, s * L:(s + 1) * L], sem_o.at[s]).wait()
    cp = pltpu.make_async_copy(patch_s, o_hbm.at[:, pl.ds(pl.multiple_of(tt * 128, 128), 128)],
                               sem_o.at[NSEG])
    cp.start()
    cp.wait()


@jax.jit
def pallas_sequential_preLN__memory_aug_infini_attn__moe_arch_mod__prompt_kernel(
    A_x: jax.Array,
    A_wq: jax.Array,
    A_wk: jax.Array,
    A_wv: jax.Array,
    A_wo: jax.Array,
    A_beta: jax.Array,
    B_x: jax.Array,
    B_w_r: jax.Array,
    B_w_gate: jax.Array,
    B_w_up: jax.Array,
    B_w_down: jax.Array,
):
    del B_x
    vmem = pl.BlockSpec(memory_space=pltpu.VMEM)
    hbm = pl.BlockSpec(memory_space=pltpu.HBM)
    out_t = pl.pallas_call(
        _kernel,
        out_shape=jax.ShapeDtypeStruct((D, S), bf16),
        in_specs=[hbm, hbm, hbm, hbm, hbm, vmem, vmem, hbm, hbm, hbm],
        out_specs=hbm,
        scratch_shapes=[
            pltpu.VMEM((NSEG, D, L), bf16),
            pltpu.VMEM((D, D), bf16),
            pltpu.VMEM((D, D), bf16),
            pltpu.VMEM((D, D), bf16),
            pltpu.VMEM((D, D), bf16),
            pltpu.VMEM((NT, 192, D), u32),
            pltpu.VMEM((D // 2, DP), u32),
            pltpu.VMEM((8, DP), f32),
            pltpu.VMEM((H + G, 8, 128), f32),
            pltpu.VMEM((D // 2, L), u32),
            pltpu.VMEM((NT, 64, L), u32),
            pltpu.VMEM((NT, L // 2, 128), u32),
            pltpu.VMEM((DP // 2, L), u32),
            pltpu.VMEM((DP, L), f32),
            pltpu.VMEM((H + G, 32, L), f32),
            pltpu.VMEM((G, 128, 128), f32),
            pltpu.VMEM((G, 256, 128), f32),
            pltpu.VMEM((G, 384, 128), f32),
            pltpu.VMEM((G, 512, 128), f32),
            pltpu.VMEM((4, G, 8, 128), f32),
            pltpu.VMEM((G, 32, 128), f32),
            pltpu.VMEM((NT, 128, 128), f32),
            pltpu.VMEM((S // 128, D // 2, 128), u32),
            pltpu.VMEM((S // 128, D // 2, 128), u32),
            pltpu.VMEM((NSEG, 8, L), f32),
            pltpu.VMEM((NSEG, D, L), bf16),
            pltpu.VMEM((D, 128), bf16),
            pltpu.VMEM((D, F), bf16),
            pltpu.VMEM((D, F), bf16),
            pltpu.VMEM((D, F), bf16),
            pltpu.SemaphoreType.DMA((NSEG,)),
            pltpu.SemaphoreType.DMA((4,)),
            pltpu.SemaphoreType.DMA((3,)),
            pltpu.SemaphoreType.DMA((NSEG + 1,)),
        ],
        compiler_params=pltpu.CompilerParams(vmem_limit_bytes=100 * 1024 * 1024),
    )(A_x.reshape(S, D).T, A_wq, A_wk, A_wv, A_wo, A_beta, B_w_r,
      B_w_gate, B_w_up, B_w_down.T)
    return out_t.T.reshape(1, S, D)
```

```python
import numpy as np
import jax
import jax.numpy as jnp
from jax import lax
import jax.experimental.pallas as pl
import jax.experimental.pallas.tpu as pltpu

S, D, H, DH = 2048, 576, 32, 18
NSEG, L = 4, 512
F = 4608
HPT = 7
NT = 5
DP = NT * 128
LOG2E = float(np.log2(np.e))
QSCALE = float(DH ** -0.5) * LOG2E
EPS_BF16 = float(np.asarray(1e-5, dtype=jnp.bfloat16).astype(np.float32))

bf16 = jnp.bfloat16
f32 = jnp.float32
u32 = jnp.uint32
G = 4
LAG = 5
STEPS = [(j, i) for j in range(4) for i in range(j + 1)]
NT_DIMS = (((1,), (1,)), ((), ()))


def _rb(x):
    return x.astype(bf16).astype(f32)


def _pack(x):
    return pltpu.bitcast(x, u32)


def _unpack(x):
    return pltpu.bitcast(x, bf16)


def _split(u):
    return tuple(pltpu.unpack_elementwise(u, index=i, packed_dtype=bf16, unpacked_dtype=f32)
                 for i in range(2))


def _merge(even, odd):
    return pltpu.pack_elementwise([even, odd], packed_dtype=bf16)


def _eo(x):
    n, m = x.shape[0] // 16, x.shape[1]
    x = x.reshape(n, 2, 8, m)
    return x[:, 0].reshape(8 * n, m), x[:, 1].reshape(8 * n, m)


def _eo_rows(u):
    n, m = u.shape[0] // 8, u.shape[1]
    even, odd = _split(u)
    x = jnp.concatenate([even.reshape(n, 8, m), odd.reshape(n, 8, m)], axis=1)
    return _pack(x.reshape(16 * n, m).astype(bf16))


def _pair_rows(u):
    n, m = u.shape[0] // 8, u.shape[1]
    x = _unpack(u).astype(f32).reshape(n, 2, 8, m)
    return _merge(x[:, 0].reshape(8 * n, m), x[:, 1].reshape(8 * n, m))


def _tree(op, x):
    parts = [x[8 * i:8 * (i + 1)] for i in range(x.shape[0] // 8)]
    while len(parts) > 1:
        parts = [op(parts[i], parts[i + 1]) if i + 1 < len(parts) else parts[i]
                 for i in range(0, len(parts), 2)]
    return parts[0]


def _colsum(pairs):
    part = jnp.concatenate([_tree(jnp.add, x) for pair in pairs for x in pair], axis=0)
    return jnp.sum(_tree(jnp.add, part), axis=0, keepdims=True)


def _head_rows(blocks):
    prev = None
    for t in range(NT):
        cur = blocks(t)
        tile = cur if t == 0 else jnp.concatenate([prev[64 - t:], cur[:64 - t]], axis=0)
        valid = min(HPT * DH, D - HPT * DH * t) // 2
        row = lax.broadcasted_iota(jnp.int32, tile.shape, 0)
        yield jnp.where(row < valid, tile, jnp.uint32(0))
        prev = cur


def _col_block_t(w_ref, i):
    if 128 * (i + 1) <= D:
        c = w_ref[:, 128 * i:128 * (i + 1)]
    else:
        c = jnp.concatenate([w_ref[:, 128 * i:], jnp.zeros((D, 128 * (i + 1) - D), bf16)], axis=1)
    return _pack(c.T)


def _row_block(w_ref, i):
    if 128 * (i + 1) <= D:
        return _pack(w_ref[128 * i:128 * (i + 1), :])
    r = _pack(w_ref[128 * i:, :])
    return jnp.concatenate([r, jnp.zeros((64 - r.shape[0], D), u32)], axis=0)


def _interleave(*gens):
    gens = list(gens)
    while gens:
        for g in list(gens):
            try:
                next(g)
            except StopIteration:
                gens.remove(g)


def _phi(t):
    return jnp.where(t > 0, t + 1.0, jnp.exp(t))


def _kernel(xt_hbm, wq_hbm, wk_hbm, wv_hbm, wo_hbm, beta_ref, wr_ref, wg_hbm, wu_hbm, wdt_hbm,
            o_hbm,
            xt_s, wq_s, wk_s, wv_s, wo_s, wc_s, wot_s, gl_s, g1_s, wr_s,
            lnt_s, q_s, k_s, vt_s, am_s, ow_s, s0_s, s1_s, s2_s, s3_s, mx_s, acc_s,
            m_s, ob0_s, ob1_s, h0_s, h1_s, h2_s, h3_s, h_s, hn_s, r_s, out_s, patch_s,
            wg_s, wu_s, wdt_s, zero_s, sem_x, sem_w, sem_f, sem_o):
    x_cp = [pltpu.make_async_copy(xt_hbm.at[:, s * L:(s + 1) * L], xt_s.at[s], sem_x.at[s])
            for s in range(NSEG)]
    w_cp = [pltpu.make_async_copy(src, dst, sem_w.at[i]) for i, (src, dst) in enumerate(
        [(wq_hbm, wq_s), (wk_hbm, wk_s), (wv_hbm, wv_s), (wo_hbm, wo_s)])]
    f_cp = [pltpu.make_async_copy(src, dst, sem_f.at[i]) for i, (src, dst) in enumerate(
        [(wg_hbm, wg_s), (wu_hbm, wu_s), (wdt_hbm, wdt_s)])]
    w_cp[0].start()
    w_cp[1].start()
    x_cp[0].start()
    w_cp[2].start()
    w_cp[3].start()

    for k in range(4):
        zero_s[k] = 0
    g = _rb(jax.nn.sigmoid(beta_ref[...].astype(f32).reshape(1, H)))
    hrow = lax.broadcasted_iota(jnp.int32, (H, DP), 0)
    fcol = lax.broadcasted_iota(jnp.int32, (H, DP), 1)
    expand = ((fcol % 128) // DH + (fcol // 128) * HPT == hrow) & (fcol % 128 < HPT * DH)
    gl_s[...] = jnp.dot(jnp.broadcast_to(g, (16, H)).astype(bf16), expand.astype(bf16),
                        preferred_element_type=f32)[0:8]
    pick = (lax.broadcasted_iota(jnp.int32, ((H + G) * 8, H), 0) // 8 - G
            == lax.broadcasted_iota(jnp.int32, ((H + G) * 8, H), 1))
    g1_s[...] = lax.dot_general(pick.astype(bf16),
                                jnp.broadcast_to(_rb(1.0 - g), (128, H)).astype(bf16), NT_DIMS,
                                preferred_element_type=f32).reshape(H + G, 8, 128)
    wr_rows = jnp.broadcast_to(wr_ref[...].reshape(1, D), (128, D)).T
    wr_s[0], wr_s[1] = _split(_pack(wr_rows))
    for ref in (s2_s, s3_s, mx_s):
        ref[...] = jnp.zeros(ref.shape, f32)
    acc_s[...] = jnp.ones(acc_s.shape, f32)

    def ln_steps(load, store):
        def chunks(k):
            return [_split(load(pl.multiple_of(zero_s[k] + 72 * c, 8)))
                    for c in range(4)]

        m = _colsum(chunks(0)) * (1.0 / D)
        yield
        sq = []
        for x in chunks(1):
            c = (x[0] - m, x[1] - m)
            sq.append((c[0] * c[0], c[1] * c[1]))
        v = _colsum(sq) * (1.0 / D)
        inv = 1.0 / _rb(jnp.sqrt(_rb(_rb(v) + EPS_BF16)))
        off = m * inv
        yield
        for c, x in enumerate(chunks(2)):
            store(72 * c, 72 * (c + 1), x, (x[0] * inv - off, x[1] * inv - off))
            if c % 2 == 1:
                yield

    def ln1_tile(s, j):
        cs = slice(128 * j, 128 * (j + 1))

        def store(lo, hi, x, y):
            lnt_s[lo:hi, cs] = _merge(*y)
        return ln_steps(
            lambda lo: _pack(xt_s[s, pl.ds(pl.multiple_of(2 * lo, 16), 144), cs]), store)

    def head_info(h):
        t = h // HPT
        r = h - HPT * t
        return t, r, pl.multiple_of(64 * t + 8 * r, 8)

    s_refs = [s0_s, s1_s, s2_s, s3_s]
    ob_tiles = [ob0_s, ob1_s]
    h_tiles = [h0_s, h1_s, h2_s, h3_s]

    def qk_step(heads, j, i, qs, mx):
        for a, (h, t, r, base) in enumerate(heads):
            kk = _unpack(k_s[t, 64 * i:64 * (i + 1), :])
            st = jnp.dot(kk, qs[a], preferred_element_type=f32)
            if i == j:
                krow = lax.broadcasted_iota(jnp.int32, (128, 128), 0)
                qcol = lax.broadcasted_iota(jnp.int32, (128, 128), 1)
                st = jnp.where(krow <= qcol, st, -1e30)
            s_refs[j][a, 128 * i:128 * (i + 1), :] = st
            m8 = _tree(jnp.maximum, st)
            mx[a] = m8 if i == 0 else jnp.maximum(mx[a], m8)
            if i == j:
                mx_s[j, a] = jnp.broadcast_to(jnp.max(mx[a], axis=0, keepdims=True), (8, 128))

    def sm_step(heads, j, i, acc, load_acc, store_acc):
        for a, (h, t, r, base) in enumerate(heads):
            st = s_refs[j][a, 128 * i:128 * (i + 1), :]
            m = mx_s[j, a]
            p = jnp.exp2(st.reshape(16, 8, 128) - m[None]).reshape(128, 128).astype(bf16)
            vw = vt_s[pl.ds(base, 16), 128 * i:128 * (i + 1)]
            vw = jnp.where(lax.broadcasted_iota(jnp.int32, (16, 128), 0) == 15,
                           jnp.uint32(0x3F803F80), vw)
            d = jnp.dot(_unpack(vw), p, preferred_element_type=f32)
            if load_acc:
                acc[a] = acc_s[a] + d
            else:
                acc[a] = d if i == 0 else acc[a] + d
            if i == j:
                scale = g1_s[h + G] / acc[a][24:32]
                ow_s[h + G, :, 128 * j:128 * (j + 1)] = acc[a] * scale[6:7]
            elif store_acc:
                acc_s[a] = acc[a]

    def sm_tail(heads):
        acc = [None] * G
        for n in range(10 - LAG, 10):
            j, i = STEPS[n]
            sm_step(heads, j, i, acc, load_acc=(n == 10 - LAG and i > 0), store_acc=False)
            yield

    def group_body(g, carry):
        cur, prev, qmask = [], [], []
        row64 = lax.broadcasted_iota(jnp.int32, (64, 128), 0)
        for a in range(G):
            h = G * g + a
            t, r, base = head_info(h)
            cur.append((h, t, r, base))
            qmask.append((row64 >= (DH // 2) * r) & (row64 < (DH // 2) * (r + 1)))
            prev.append((h - G,) + head_info(jnp.maximum(h - G, 0)))
        tail = sm_tail(prev)
        acc = [None] * G
        qs, mx = None, [None] * G
        for n in range(10):
            j, i = STEPS[n]
            if i == 0:
                qs = [_unpack(jnp.where(qmask[a], q_s[cur[a][1], :, 128 * j:128 * (j + 1)],
                                        jnp.uint32(0))) for a in range(G)]
            qk_step(cur, j, i, qs, mx)
            if n < LAG:
                next(tail)
            else:
                jj, ii = STEPS[n - LAG]
                sm_step(cur, jj, ii, acc, load_acc=False, store_acc=(n == 9))
        return carry

    def project(t, first=False):
        rows = 64 if t < NT - 1 else 40
        w = wc_s[t]
        w = jnp.concatenate([w[0:rows], w[64:64 + rows], w[128:128 + rows]], axis=0)
        qkv = jnp.dot(_unpack(w), _unpack(lnt_s[...]), preferred_element_type=f32)
        n = 2 * rows

        def full(u):
            return u if rows == 64 else jnp.concatenate(
                [u, jnp.zeros((64 - rows, L), u32)], axis=0)

        qf, kf, vf = _eo(qkv[0:n]), _eo(qkv[n:2 * n]), _eo(qkv[2 * n:3 * n])
        q_s[t] = full(_merge(qf[0] * QSCALE, qf[1] * QSCALE))
        k_s[t] = _pack(_unpack(full(_merge(*kf))).T)
        vt = full(_merge(*vf))
        vt_s[64 * t:64 * (t + 1), :] = vt
        pq = _unpack(full(_merge(_phi(qf[0]), _phi(qf[1]))))
        pk = _unpack(full(_merge(_phi(kf[0]), _phi(kf[1]))))
        vone = jnp.where(lax.broadcasted_iota(jnp.int32, (64, L), 0) == 63,
                         jnp.uint32(0x3F803F80), vt)
        upd = lax.dot_general(_unpack(vone), pk, NT_DIMS, preferred_element_type=f32)
        if first:
            am_s[128 * t:128 * (t + 1), :] = jnp.zeros((128, L), f32)
            m_s[t] = upd
            return
        erow = lax.broadcasted_iota(jnp.int32, (128, 128), 0)
        dcol = lax.broadcasted_iota(jnp.int32, (128, 128), 1)
        bd_mask = (erow // DH == dcol // DH) & (dcol < HPT * DH)
        zrow = lax.broadcasted_iota(jnp.int32, (16, 128), 0)
        zcol = lax.broadcasted_iota(jnp.int32, (16, 128), 1)
        z_mask = (zcol // DH == zrow) & (zcol < HPT * DH)
        mt = m_s[t]
        mb = jnp.where(bd_mask, mt * gl_s[0:1, 128 * t:128 * (t + 1)], 0.0)
        zb = jnp.where(z_mask, jnp.broadcast_to(mt[126:127, :], (16, 128)), 0.0)
        nd = jnp.dot(jnp.concatenate([mb, zb], axis=0).astype(bf16), pq,
                     preferred_element_type=f32)
        inv = 1.0 / (nd[128:136] + 1e-6)
        row8 = lax.broadcasted_iota(jnp.int32, (8, L), 0)
        bro = [jnp.broadcast_to(inv[a:a + 1], (8, L)) for a in range(HPT)]
        for u in range(16):
            ha, hb = (8 * u) // DH, min((8 * u + 7) // DH, HPT - 1)
            sc = bro[ha] if ha == hb else jnp.where(row8 < DH * hb - 8 * u, bro[ha], bro[hb])
            am_s[128 * t + 8 * u:128 * t + 8 * (u + 1), :] = nd[8 * u:8 * (u + 1)] * sc
        m_s[t] = mt + upd

    def mix_tile(j):
        cs = slice(128 * j, 128 * (j + 1))
        row8 = lax.broadcasted_iota(jnp.int32, (8, 128), 0)
        parts = []
        for t in range(NT):
            for u in range(16):
                rr, half = u // 2, u % 2
                h = HPT * t + rr
                cut = 2 * rr - 8 * half
                lo_ok, hi_ok = (rr > 0 and h - 1 < H), (rr < HPT and h < H)
                lo = ow_s[h - 1 + G, 16 + 8 * half:24 + 8 * half, cs] if lo_ok else None
                hi = ow_s[h + G, 8 * half:8 * half + 8, cs] if hi_ok else None
                if cut <= 0 or not lo_ok:
                    dp = hi
                elif cut >= 8 or not hi_ok:
                    dp = lo
                else:
                    dp = jnp.where(row8 >= cut, hi, lo)
                am = am_s[128 * t + 8 * u:128 * t + 8 * (u + 1), cs]
                parts.append(am if dp is None else am + dp)
            ob_tiles[j % 2][64 * t:64 * (t + 1), :] = _merge(
                jnp.concatenate(parts[0::2], axis=0), jnp.concatenate(parts[1::2], axis=0))
            parts = []
            if t % 2 == 1:
                yield
        yield

    def out_proj_tile(s, j):
        cs = slice(128 * j, 128 * (j + 1))
        for c in range(4):
            w = _unpack(wot_s[72 * c:72 * (c + 1), :])
            attn = _eo(jnp.dot(w, _unpack(ob_tiles[j % 2][...]), preferred_element_type=f32))
            x = _split(_pack(xt_s[s, 144 * c:144 * (c + 1), cs]))
            hb = _merge(x[0] + attn[0], x[1] + attn[1])
            h_tiles[j][72 * c:72 * (c + 1), :] = hb
            h_s[4 * s + j, 72 * c:72 * (c + 1), :] = hb
            yield

    def ln2_tile(s, j):
        cs = slice(128 * j, 128 * (j + 1))
        score = []

        def store(lo, hi, h, hn):
            out_s[s, 2 * lo:2 * hi, cs] = _unpack(_merge(h[0] + hn[0], h[1] + hn[1]))
            hn_s[4 * s + j, lo:hi, :] = _merge(*hn)
            score.append(_tree(jnp.add, hn[0] * wr_s[0, lo:hi])
                         + _tree(jnp.add, hn[1] * wr_s[1, lo:hi]))
            if hi == D // 2:
                r_s[s, :, cs] = (score[0] + score[1]) + (score[2] + score[3])
        return ln_steps(lambda lo: h_tiles[j][pl.ds(lo, 72), :], store)

    x_cp[0].wait()
    w_cp[0].wait()
    w_cp[1].wait()
    w_cp[2].wait()
    for s in range(1, NSEG):
        x_cp[s].start()
    wq_t = _head_rows(lambda i: _col_block_t(wq_s, i))
    wk_t = _head_rows(lambda i: _col_block_t(wk_s, i))
    wv_t = _head_rows(lambda i: _col_block_t(wv_s, i))
    wo_t = _head_rows(lambda i: _row_block(wo_s, i))

    def first_weights():
        for rows, tiles in ((0, wq_t), (64, wk_t), (128, wv_t)):
            wc_s[0, rows:rows + 64, :] = _eo_rows(next(tiles))
            yield

    _interleave(first_weights(), *[ln1_tile(0, j) for j in range(4)])
    w_cp[3].wait()
    for c in f_cp:
        c.start()
    for t in range(NT):
        if t + 1 < NT:
            wc_s[t + 1] = jnp.concatenate(
                [_eo_rows(next(wq_t)), _eo_rows(next(wk_t)), _eo_rows(next(wv_t))], axis=0)
        project(t, first=True)
        wot_s[:, 128 * t:128 * (t + 1)] = _eo_rows(_pack(_unpack(_pair_rows(next(wo_t))).T))

    def segment(s, last):
        if not last:
            pltpu.make_async_copy(xt_s.at[s + 1], xt_s.at[s + 1], sem_x.at[s + 1]).wait()

        lax.fori_loop(0, H // G, group_body, 0, unroll=2)

        tail = sm_tail([(h, h // HPT, h % HPT, 64 * (h // HPT) + 8 * (h % HPT))
                        for h in range(H - G, H)])
        _interleave(mix_tile(0), tail)
        for j in range(4):
            gens = [out_proj_tile(s, j)]
            if not last:
                gens.append(ln1_tile(s + 1, j))
            if j < 3:
                gens.append(mix_tile(j + 1))
            if j > 0:
                gens.append(ln2_tile(s, j - 1))
            _interleave(*gens)

        def finish():
            yield from ln2_tile(s, 3)
            lo = s * L if last else pl.multiple_of(s * L, L)
            pltpu.make_async_copy(out_s.at[s], o_hbm.at[:, pl.ds(lo, L)], sem_o.at[s]).start()

        def next_projections():
            for t in range(NT):
                project(t)
                yield

        if last:
            _interleave(finish())
        else:
            _interleave(next_projections(), finish())

    def segment_body(s, carry):
        segment(s, False)
        return carry

    lax.fori_loop(0, NSEG - 1, segment_body, 0)
    segment(NSEG - 1, True)

    rall = jnp.concatenate([_rb(jnp.sum(r_s[s], axis=0, keepdims=True))
                            for s in range(NSEG)], axis=0)
    rmax = jnp.max(rall)
    pos = (lax.broadcasted_iota(jnp.int32, (NSEG, L), 0) * L
           + lax.broadcasted_iota(jnp.int32, (NSEG, L), 1))
    idx = jnp.clip(jnp.min(jnp.where(rall == rmax, pos, S)), 0, S - 1)
    tt = idx // 128
    ln_sel = idx - tt * 128
    rsel = _rb(jax.nn.sigmoid(jnp.full((1, 1), rmax, f32)))
    hn_t = _unpack(hn_s[tt])
    h_t = _unpack(h_s[tt]).astype(f32)
    onehot = (lax.broadcasted_iota(jnp.int32, (16, 128), 1) == ln_sel).astype(bf16)
    xsel = lax.dot_general(onehot, hn_t, NT_DIMS, preferred_element_type=f32).astype(bf16)

    f_cp[0].wait()
    f_cp[1].wait()
    gate = _rb(jnp.dot(xsel, wg_s[...], preferred_element_type=f32))
    up = _rb(jnp.dot(xsel, wu_s[...], preferred_element_type=f32))
    gu = (_rb(gate * jax.nn.sigmoid(gate)) * up).astype(bf16)
    f_cp[2].wait()
    y = _rb(lax.dot_general(gu, wdt_s[...], NT_DIMS, preferred_element_type=f32))
    y = _rb(y * rsel)
    yt = jnp.broadcast_to(y[0:1], (128, D)).T
    upd = jnp.where(lax.broadcasted_iota(jnp.int32, (D, 128), 1) == ln_sel, yt, 0.0)
    patch_s[...] = (h_t + _rb(hn_t.astype(f32) + upd)).astype(bf16)
    for s in range(NSEG):
        pltpu.make_async_copy(out_s.at[s], o_hbm.at[:, s * L:(s + 1) * L], sem_o.at[s]).wait()
    cp = pltpu.make_async_copy(patch_s, o_hbm.at[:, pl.ds(pl.multiple_of(tt * 128, 128), 128)],
                               sem_o.at[NSEG])
    cp.start()
    cp.wait()


@jax.jit
def pallas_sequential_preLN__memory_aug_infini_attn__moe_arch_mod__prompt_kernel(
    A_x: jax.Array,
    A_wq: jax.Array,
    A_wk: jax.Array,
    A_wv: jax.Array,
    A_wo: jax.Array,
    A_beta: jax.Array,
    B_x: jax.Array,
    B_w_r: jax.Array,
    B_w_gate: jax.Array,
    B_w_up: jax.Array,
    B_w_down: jax.Array,
):
    del B_x
    vmem = pl.BlockSpec(memory_space=pltpu.VMEM)
    hbm = pl.BlockSpec(memory_space=pltpu.HBM)
    out_t = pl.pallas_call(
        _kernel,
        out_shape=jax.ShapeDtypeStruct((D, S), bf16),
        in_specs=[hbm, hbm, hbm, hbm, hbm, vmem, vmem, hbm, hbm, hbm],
        out_specs=hbm,
        scratch_shapes=[
            pltpu.VMEM((NSEG, D, L), bf16),
            pltpu.VMEM((D, D), bf16),
            pltpu.VMEM((D, D), bf16),
            pltpu.VMEM((D, D), bf16),
            pltpu.VMEM((D, D), bf16),
            pltpu.VMEM((NT, 192, D), u32),
            pltpu.VMEM((D // 2, DP), u32),
            pltpu.VMEM((8, DP), f32),
            pltpu.VMEM((H + G, 8, 128), f32),
            pltpu.VMEM((2, D // 2, 128), f32),
            pltpu.VMEM((D // 2, L), u32),
            pltpu.VMEM((NT, 64, L), u32),
            pltpu.VMEM((NT, L // 2, 128), u32),
            pltpu.VMEM((DP // 2, L), u32),
            pltpu.VMEM((DP, L), f32),
            pltpu.VMEM((H + G, 32, L), f32),
            pltpu.VMEM((G, 128, 128), f32),
            pltpu.VMEM((G, 256, 128), f32),
            pltpu.VMEM((G, 384, 128), f32),
            pltpu.VMEM((G, 512, 128), f32),
            pltpu.VMEM((4, G, 8, 128), f32),
            pltpu.VMEM((G, 32, 128), f32),
            pltpu.VMEM((NT, 128, 128), f32),
            *[pltpu.VMEM((DP // 2, 128), u32)] * 2,
            *[pltpu.VMEM((D // 2, 128), u32)] * 4,
            pltpu.VMEM((S // 128, D // 2, 128), u32),
            pltpu.VMEM((S // 128, D // 2, 128), u32),
            pltpu.VMEM((NSEG, 8, L), f32),
            pltpu.VMEM((NSEG, D, L), bf16),
            pltpu.VMEM((D, 128), bf16),
            pltpu.VMEM((D, F), bf16),
            pltpu.VMEM((D, F), bf16),
            pltpu.VMEM((D, F), bf16),
            pltpu.SMEM((4,), jnp.int32),
            pltpu.SemaphoreType.DMA((NSEG,)),
            pltpu.SemaphoreType.DMA((4,)),
            pltpu.SemaphoreType.DMA((3,)),
            pltpu.SemaphoreType.DMA((NSEG + 1,)),
        ],
        compiler_params=pltpu.CompilerParams(vmem_limit_bytes=100 * 1024 * 1024),
    )(A_x.reshape(S, D).T, A_wq, A_wk, A_wv, A_wo, A_beta, B_w_r,
      B_w_gate, B_w_up, B_w_down.T)
    return out_t.T.reshape(1, S, D)
```

```python
import numpy as np
import jax
import jax.numpy as jnp
from jax import lax
import jax.experimental.pallas as pl
import jax.experimental.pallas.tpu as pltpu

S, D, H, DH = 2048, 576, 32, 18
NSEG, L = 4, 512
F = 4608
HPT = 7
NT = 5
DP = NT * 128
LOG2E = float(np.log2(np.e))
QSCALE = float(DH ** -0.5) * LOG2E
EPS_BF16 = float(np.asarray(1e-5, dtype=jnp.bfloat16).astype(np.float32))

bf16 = jnp.bfloat16
f32 = jnp.float32
u32 = jnp.uint32
G = 4
LAG = 5
STEPS = [(j, i) for j in range(4) for i in range(j + 1)]
NT_DIMS = (((1,), (1,)), ((), ()))


def _rb(x):
    return x.astype(bf16).astype(f32)


def _pack(x):
    return pltpu.bitcast(x, u32)


def _unpack(x):
    return pltpu.bitcast(x, bf16)


def _split(u):
    return tuple(pltpu.unpack_elementwise(u, index=i, packed_dtype=bf16, unpacked_dtype=f32)
                 for i in range(2))


def _merge(even, odd):
    return pltpu.pack_elementwise([even, odd], packed_dtype=bf16)


def _eo(x):
    n, m = x.shape[0] // 16, x.shape[1]
    x = x.reshape(n, 2, 8, m)
    return x[:, 0].reshape(8 * n, m), x[:, 1].reshape(8 * n, m)


def _eo_rows(u):
    n, m = u.shape[0] // 8, u.shape[1]
    even, odd = _split(u)
    x = jnp.concatenate([even.reshape(n, 8, m), odd.reshape(n, 8, m)], axis=1)
    return _pack(x.reshape(16 * n, m).astype(bf16))


def _pair_rows(u):
    n, m = u.shape[0] // 8, u.shape[1]
    x = _unpack(u).astype(f32).reshape(n, 2, 8, m)
    return _merge(x[:, 0].reshape(8 * n, m), x[:, 1].reshape(8 * n, m))


def _tree(op, x):
    parts = [x[8 * i:8 * (i + 1)] for i in range(x.shape[0] // 8)]
    while len(parts) > 1:
        parts = [op(parts[i], parts[i + 1]) if i + 1 < len(parts) else parts[i]
                 for i in range(0, len(parts), 2)]
    return parts[0]


def _colsum(pairs):
    part = jnp.concatenate([_tree(jnp.add, x) for pair in pairs for x in pair], axis=0)
    return jnp.sum(_tree(jnp.add, part), axis=0, keepdims=True)


def _head_rows(blocks):
    prev = None
    for t in range(NT):
        cur = blocks(t)
        tile = cur if t == 0 else jnp.concatenate([prev[64 - t:], cur[:64 - t]], axis=0)
        valid = min(HPT * DH, D - HPT * DH * t) // 2
        row = lax.broadcasted_iota(jnp.int32, tile.shape, 0)
        yield jnp.where(row < valid, tile, jnp.uint32(0))
        prev = cur


def _col_block_t(w_ref, i):
    if 128 * (i + 1) <= D:
        c = w_ref[:, 128 * i:128 * (i + 1)]
    else:
        c = jnp.concatenate([w_ref[:, 128 * i:], jnp.zeros((D, 128 * (i + 1) - D), bf16)], axis=1)
    return _pack(c.T)


def _row_block(w_ref, i):
    if 128 * (i + 1) <= D:
        return _pack(w_ref[128 * i:128 * (i + 1), :])
    r = _pack(w_ref[128 * i:, :])
    return jnp.concatenate([r, jnp.zeros((64 - r.shape[0], D), u32)], axis=0)


def _interleave(*gens):
    gens = list(gens)
    while gens:
        for g in list(gens):
            try:
                next(g)
            except StopIteration:
                gens.remove(g)


def _phi(t):
    return jnp.where(t > 0, t + 1.0, jnp.exp(t))


def _kernel(xt_hbm, wq_hbm, wk_hbm, wv_hbm, wo_hbm, beta_ref, wr_ref, wg_hbm, wu_hbm, wdt_hbm,
            o_hbm,
            xt_s, wq_s, wk_s, wv_s, wo_s, wc_s, wot_s, gl_s, g1_s, wr_s,
            lnt_s, q_s, k_s, vt_s, pq_s, pk_s, am_s, ow_s, s0_s, s1_s, s2_s, s3_s, mx_s, acc_s,
            m_s, ob0_s, ob1_s, h0_s, h1_s, h2_s, h3_s, h_s, hn_s, r_s, out_s, patch_s,
            wg_s, wu_s, wdt_s, zero_s, sem_x, sem_w, sem_f, sem_o):
    def cols(i):
        return slice(128 * i, min(128 * (i + 1), D))

    x0_cp = [pltpu.make_async_copy(xt_hbm.at[:, cols(j)], xt_s.at[0, :, cols(j)], sem_x.at[j])
             for j in range(4)]
    x_cp = [None] + [pltpu.make_async_copy(xt_hbm.at[:, s * L:(s + 1) * L], xt_s.at[s],
                                           sem_x.at[3 + s]) for s in range(1, NSEG)]
    w_cp = [[pltpu.make_async_copy(src.at[:, cols(i)], dst.at[:, cols(i)], sem_w.at[3 * i + n])
             for n, (src, dst) in enumerate([(wq_hbm, wq_s), (wk_hbm, wk_s), (wv_hbm, wv_s)])]
            for i in range(NT)]
    wo_cp = pltpu.make_async_copy(wo_hbm, wo_s, sem_w.at[3 * NT])
    f_cp = [pltpu.make_async_copy(src, dst, sem_f.at[i]) for i, (src, dst) in enumerate(
        [(wg_hbm, wg_s), (wu_hbm, wu_s), (wdt_hbm, wdt_s)])]
    for c in x0_cp + w_cp[0]:
        c.start()
    for i in range(1, NT):
        for c in w_cp[i]:
            c.start()
    wo_cp.start()

    for k in range(4):
        zero_s[k] = 0
    g = _rb(jax.nn.sigmoid(beta_ref[...].astype(f32).reshape(1, H)))
    hrow = lax.broadcasted_iota(jnp.int32, (H, DP), 0)
    fcol = lax.broadcasted_iota(jnp.int32, (H, DP), 1)
    expand = ((fcol % 128) // DH + (fcol // 128) * HPT == hrow) & (fcol % 128 < HPT * DH)
    gl_s[...] = jnp.dot(jnp.broadcast_to(g, (16, H)).astype(bf16), expand.astype(bf16),
                        preferred_element_type=f32)[0:8]
    pick = (lax.broadcasted_iota(jnp.int32, ((H + G) * 8, H), 0) // 8 - G
            == lax.broadcasted_iota(jnp.int32, ((H + G) * 8, H), 1))
    g1_s[...] = lax.dot_general(pick.astype(bf16),
                                jnp.broadcast_to(_rb(1.0 - g), (128, H)).astype(bf16), NT_DIMS,
                                preferred_element_type=f32).reshape(H + G, 8, 128)
    wr_rows = jnp.broadcast_to(wr_ref[...].reshape(1, D), (128, D)).T
    wr_s[0], wr_s[1] = _split(_pack(wr_rows))
    m_s[...] = jnp.zeros(m_s.shape, f32)
    for ref in (s2_s, s3_s, mx_s):
        ref[...] = jnp.zeros(ref.shape, f32)
    acc_s[...] = jnp.ones(acc_s.shape, f32)

    def ln_steps(load, store):
        def chunks(k):
            return [_split(load(pl.multiple_of(zero_s[k] + 72 * c, 8)))
                    for c in range(4)]

        m = _colsum(chunks(0)) * (1.0 / D)
        yield
        sq = []
        for x in chunks(1):
            c = (x[0] - m, x[1] - m)
            sq.append((c[0] * c[0], c[1] * c[1]))
        v = _colsum(sq) * (1.0 / D)
        inv = 1.0 / _rb(jnp.sqrt(_rb(_rb(v) + EPS_BF16)))
        off = m * inv
        yield
        for c, x in enumerate(chunks(2)):
            store(72 * c, 72 * (c + 1), x, (x[0] * inv - off, x[1] * inv - off))
            if c % 2 == 1:
                yield

    def ln1_tile(s, j):
        cs = slice(128 * j, 128 * (j + 1))

        def store(lo, hi, x, y):
            lnt_s[lo:hi, cs] = _merge(*y)
        return ln_steps(
            lambda lo: _pack(xt_s[s, pl.ds(pl.multiple_of(2 * lo, 16), 144), cs]), store)

    def head_info(h):
        t = h // HPT
        r = h - HPT * t
        return t, r, pl.multiple_of(64 * t + 8 * r, 8)

    s_refs = [s0_s, s1_s, s2_s, s3_s]
    ob_tiles = [ob0_s, ob1_s]
    h_tiles = [h0_s, h1_s, h2_s, h3_s]

    def qk_step(heads, j, i, qs, mx):
        for a, (h, t, r, base) in enumerate(heads):
            kk = _unpack(k_s[t, 64 * i:64 * (i + 1), :])
            st = jnp.dot(kk, qs[a], preferred_element_type=f32)
            if i == j:
                krow = lax.broadcasted_iota(jnp.int32, (128, 128), 0)
                qcol = lax.broadcasted_iota(jnp.int32, (128, 128), 1)
                st = jnp.where(krow <= qcol, st, -1e30)
            s_refs[j][a, 128 * i:128 * (i + 1), :] = st
            m8 = _tree(jnp.maximum, st)
            mx[a] = m8 if i == 0 else jnp.maximum(mx[a], m8)
            if i == j:
                mx_s[j, a] = jnp.broadcast_to(jnp.max(mx[a], axis=0, keepdims=True), (8, 128))

    def sm_step(heads, j, i, acc, load_acc, store_acc):
        for a, (h, t, r, base) in enumerate(heads):
            st = s_refs[j][a, 128 * i:128 * (i + 1), :]
            m = mx_s[j, a]
            p = jnp.exp2(st.reshape(16, 8, 128) - m[None]).reshape(128, 128).astype(bf16)
            vw = vt_s[pl.ds(base, 16), 128 * i:128 * (i + 1)]
            vw = jnp.where(lax.broadcasted_iota(jnp.int32, (16, 128), 0) == 15,
                           jnp.uint32(0x3F803F80), vw)
            d = jnp.dot(_unpack(vw), p, preferred_element_type=f32)
            if load_acc:
                acc[a] = acc_s[a] + d
            else:
                acc[a] = d if i == 0 else acc[a] + d
            if i == j:
                scale = g1_s[h + G] / acc[a][24:32]
                ow_s[h + G, :, 128 * j:128 * (j + 1)] = acc[a] * scale[6:7]
            elif store_acc:
                acc_s[a] = acc[a]

    def sm_tail(heads):
        acc = [None] * G
        for n in range(10 - LAG, 10):
            j, i = STEPS[n]
            sm_step(heads, j, i, acc, load_acc=(n == 10 - LAG and i > 0), store_acc=False)
            yield

    def group_body(g, carry):
        cur, prev, qmask = [], [], []
        row64 = lax.broadcasted_iota(jnp.int32, (64, 128), 0)
        for a in range(G):
            h = G * g + a
            t, r, base = head_info(h)
            cur.append((h, t, r, base))
            qmask.append((row64 >= (DH // 2) * r) & (row64 < (DH // 2) * (r + 1)))
            prev.append((h - G,) + head_info(jnp.maximum(h - G, 0)))
        tail = sm_tail(prev)
        acc = [None] * G
        qs, mx = None, [None] * G
        for n in range(10):
            j, i = STEPS[n]
            if i == 0:
                qs = [_unpack(jnp.where(qmask[a], q_s[cur[a][1], :, 128 * j:128 * (j + 1)],
                                        jnp.uint32(0))) for a in range(G)]
            qk_step(cur, j, i, qs, mx)
            if n < LAG:
                next(tail)
            else:
                jj, ii = STEPS[n - LAG]
                sm_step(cur, jj, ii, acc, load_acc=False, store_acc=(n == 9))
        return carry

    def project(t):
        rows = 64 if t < NT - 1 else 40
        w = wc_s[t]
        w = jnp.concatenate([w[0:rows], w[64:64 + rows], w[128:128 + rows]], axis=0)
        qkv = jnp.dot(_unpack(w), _unpack(lnt_s[...]), preferred_element_type=f32)
        n = 2 * rows

        def full(u):
            return u if rows == 64 else jnp.concatenate(
                [u, jnp.zeros((64 - rows, L), u32)], axis=0)

        qf, kf, vf = _eo(qkv[0:n]), _eo(qkv[n:2 * n]), _eo(qkv[2 * n:3 * n])
        q_s[t] = full(_merge(qf[0] * QSCALE, qf[1] * QSCALE))
        k_s[t] = _pack(_unpack(full(_merge(*kf))).T)
        vt = full(_merge(*vf))
        vt_s[64 * t:64 * (t + 1), :] = vt
        pq_s[t] = full(_merge(_phi(qf[0]), _phi(qf[1])))
        pk_s[t] = full(_merge(_phi(kf[0]), _phi(kf[1])))

    def memory_read(t):
        erow = lax.broadcasted_iota(jnp.int32, (128, 128), 0)
        dcol = lax.broadcasted_iota(jnp.int32, (128, 128), 1)
        bd_mask = (erow // DH == dcol // DH) & (dcol < HPT * DH)
        zrow = lax.broadcasted_iota(jnp.int32, (16, 128), 0)
        zcol = lax.broadcasted_iota(jnp.int32, (16, 128), 1)
        z_mask = (zcol // DH == zrow) & (zcol < HPT * DH)
        mt = m_s[t]
        pq = _unpack(pq_s[t])
        mb = jnp.where(bd_mask, mt * gl_s[0:1, 128 * t:128 * (t + 1)], 0.0)
        zb = jnp.where(z_mask, jnp.broadcast_to(mt[126:127, :], (16, 128)), 0.0)
        nd = jnp.dot(jnp.concatenate([mb, zb], axis=0).astype(bf16), pq,
                     preferred_element_type=f32)
        inv = 1.0 / (nd[128:136] + 1e-6)
        row8 = lax.broadcasted_iota(jnp.int32, (8, L), 0)
        bro = [jnp.broadcast_to(inv[a:a + 1], (8, L)) for a in range(HPT)]
        for u in range(16):
            ha, hb = (8 * u) // DH, min((8 * u + 7) // DH, HPT - 1)
            sc = bro[ha] if ha == hb else jnp.where(row8 < DH * hb - 8 * u, bro[ha], bro[hb])
            am_s[128 * t + 8 * u:128 * t + 8 * (u + 1), :] = nd[8 * u:8 * (u + 1)] * sc

    def memory_update(t):
        vone = jnp.where(lax.broadcasted_iota(jnp.int32, (64, L), 0) == 63,
                         jnp.uint32(0x3F803F80), vt_s[64 * t:64 * (t + 1), :])
        m_s[t] += lax.dot_general(_unpack(vone), _unpack(pk_s[t]), NT_DIMS,
                                  preferred_element_type=f32)

    def mix_tile(j):
        cs = slice(128 * j, 128 * (j + 1))
        row8 = lax.broadcasted_iota(jnp.int32, (8, 128), 0)
        parts = []
        for t in range(NT):
            for u in range(16):
                rr, half = u // 2, u % 2
                h = HPT * t + rr
                cut = 2 * rr - 8 * half
                lo_ok, hi_ok = (rr > 0 and h - 1 < H), (rr < HPT and h < H)
                lo = ow_s[h - 1 + G, 16 + 8 * half:24 + 8 * half, cs] if lo_ok else None
                hi = ow_s[h + G, 8 * half:8 * half + 8, cs] if hi_ok else None
                if cut <= 0 or not lo_ok:
                    dp = hi
                elif cut >= 8 or not hi_ok:
                    dp = lo
                else:
                    dp = jnp.where(row8 >= cut, hi, lo)
                am = am_s[128 * t + 8 * u:128 * t + 8 * (u + 1), cs]
                parts.append(am if dp is None else am + dp)
            ob_tiles[j % 2][64 * t:64 * (t + 1), :] = _merge(
                jnp.concatenate(parts[0::2], axis=0), jnp.concatenate(parts[1::2], axis=0))
            parts = []
            if t % 2 == 1:
                yield
        yield

    def out_proj_tile(s, j):
        cs = slice(128 * j, 128 * (j + 1))
        for c in range(4):
            w = _unpack(wot_s[72 * c:72 * (c + 1), :])
            attn = _eo(jnp.dot(w, _unpack(ob_tiles[j % 2][...]), preferred_element_type=f32))
            x = _split(_pack(xt_s[s, 144 * c:144 * (c + 1), cs]))
            hb = _merge(x[0] + attn[0], x[1] + attn[1])
            h_tiles[j][72 * c:72 * (c + 1), :] = hb
            h_s[4 * s + j, 72 * c:72 * (c + 1), :] = hb
            yield

    def ln2_tile(s, j):
        cs = slice(128 * j, 128 * (j + 1))
        score = []

        def store(lo, hi, h, hn):
            out_s[s, 2 * lo:2 * hi, cs] = _unpack(_merge(h[0] + hn[0], h[1] + hn[1]))
            hn_s[4 * s + j, lo:hi, :] = _merge(*hn)
            score.append(_tree(jnp.add, hn[0] * wr_s[0, lo:hi])
                         + _tree(jnp.add, hn[1] * wr_s[1, lo:hi]))
            if hi == D // 2:
                r_s[s, :, cs] = (score[0] + score[1]) + (score[2] + score[3])
        return ln_steps(lambda lo: h_tiles[j][pl.ds(lo, 72), :], store)

    wq_t = _head_rows(lambda i: _col_block_t(wq_s, i))
    wk_t = _head_rows(lambda i: _col_block_t(wk_s, i))
    wv_t = _head_rows(lambda i: _col_block_t(wv_s, i))
    wo_t = _head_rows(lambda i: _row_block(wo_s, i))

    def first_weights():
        for rows, tiles in ((0, wq_t), (64, wk_t), (128, wv_t)):
            wc_s[0, rows:rows + 64, :] = _eo_rows(next(tiles))
            yield

    def first_ln(j):
        x0_cp[j].wait()
        yield from ln1_tile(0, j)

    for j in range(4):
        _interleave(first_ln(j))
    for c in w_cp[0]:
        c.wait()
    _interleave(first_weights())
    for c in [c for i in range(1, NT) for c in w_cp[i]] + [wo_cp]:
        c.wait()
    for c in x_cp[1:] + f_cp:
        c.start()
    for t in range(NT):
        if t + 1 < NT:
            wc_s[t + 1] = jnp.concatenate(
                [_eo_rows(next(wq_t)), _eo_rows(next(wk_t)), _eo_rows(next(wv_t))], axis=0)
        project(t)
        wot_s[:, 128 * t:128 * (t + 1)] = _eo_rows(_pack(_unpack(_pair_rows(next(wo_t))).T))

    def segment(s, last):
        if not last:
            pltpu.make_async_copy(xt_s.at[s + 1], xt_s.at[s + 1], sem_x.at[4 + s]).wait()

        lax.fori_loop(0, H // G, group_body, 0, unroll=2)

        tail = sm_tail([(h, h // HPT, h % HPT, 64 * (h // HPT) + 8 * (h % HPT))
                        for h in range(H - G, H)])
        def reads():
            for t in range(NT):
                memory_read(t)
                yield

        def updates():
            for t in range(NT):
                memory_update(t)
                yield

        _interleave(reads(), tail)
        _interleave(mix_tile(0), *([] if last else [updates()]))
        for j in range(4):
            gens = [out_proj_tile(s, j)]
            if not last:
                gens.append(ln1_tile(s + 1, j))
            if j < 3:
                gens.append(mix_tile(j + 1))
            if j > 0:
                gens.append(ln2_tile(s, j - 1))
            _interleave(*gens)

        def finish():
            yield from ln2_tile(s, 3)
            lo = s * L if last else pl.multiple_of(s * L, L)
            pltpu.make_async_copy(out_s.at[s], o_hbm.at[:, pl.ds(lo, L)], sem_o.at[s]).start()

        def next_projections():
            for t in range(NT):
                project(t)
                yield

        if last:
            _interleave(finish())
        else:
            _interleave(next_projections(), finish())

    def segment_body(s, carry):
        segment(s, False)
        return carry

    lax.fori_loop(0, NSEG - 1, segment_body, 0)
    segment(NSEG - 1, True)

    rall = jnp.concatenate([_rb(jnp.sum(r_s[s], axis=0, keepdims=True))
                            for s in range(NSEG)], axis=0)
    rmax = jnp.max(rall)
    pos = (lax.broadcasted_iota(jnp.int32, (NSEG, L), 0) * L
           + lax.broadcasted_iota(jnp.int32, (NSEG, L), 1))
    idx = jnp.clip(jnp.min(jnp.where(rall == rmax, pos, S)), 0, S - 1)
    tt = idx // 128
    ln_sel = idx - tt * 128
    rsel = _rb(jax.nn.sigmoid(jnp.full((1, 1), rmax, f32)))
    hn_t = _unpack(hn_s[tt])
    h_t = _unpack(h_s[tt]).astype(f32)
    onehot = (lax.broadcasted_iota(jnp.int32, (16, 128), 1) == ln_sel).astype(bf16)
    xsel = lax.dot_general(onehot, hn_t, NT_DIMS, preferred_element_type=f32).astype(bf16)

    f_cp[0].wait()
    f_cp[1].wait()
    gate = _rb(jnp.dot(xsel, wg_s[...], preferred_element_type=f32))
    up = _rb(jnp.dot(xsel, wu_s[...], preferred_element_type=f32))
    gu = (_rb(gate * jax.nn.sigmoid(gate)) * up).astype(bf16)
    f_cp[2].wait()
    y = _rb(lax.dot_general(gu, wdt_s[...], NT_DIMS, preferred_element_type=f32))
    y = _rb(y * rsel)
    yt = jnp.broadcast_to(y[0:1], (128, D)).T
    upd = jnp.where(lax.broadcasted_iota(jnp.int32, (D, 128), 1) == ln_sel, yt, 0.0)
    patch_s[...] = (h_t + _rb(hn_t.astype(f32) + upd)).astype(bf16)
    for s in range(NSEG):
        pltpu.make_async_copy(out_s.at[s], o_hbm.at[:, s * L:(s + 1) * L], sem_o.at[s]).wait()
    cp = pltpu.make_async_copy(patch_s, o_hbm.at[:, pl.ds(pl.multiple_of(tt * 128, 128), 128)],
                               sem_o.at[NSEG])
    cp.start()
    cp.wait()


@jax.jit
def pallas_sequential_preLN__memory_aug_infini_attn__moe_arch_mod__prompt_kernel(
    A_x: jax.Array,
    A_wq: jax.Array,
    A_wk: jax.Array,
    A_wv: jax.Array,
    A_wo: jax.Array,
    A_beta: jax.Array,
    B_x: jax.Array,
    B_w_r: jax.Array,
    B_w_gate: jax.Array,
    B_w_up: jax.Array,
    B_w_down: jax.Array,
):
    del B_x
    vmem = pl.BlockSpec(memory_space=pltpu.VMEM)
    hbm = pl.BlockSpec(memory_space=pltpu.HBM)
    out_t = pl.pallas_call(
        _kernel,
        out_shape=jax.ShapeDtypeStruct((D, S), bf16),
        in_specs=[hbm, hbm, hbm, hbm, hbm, vmem, vmem, hbm, hbm, hbm],
        out_specs=hbm,
        scratch_shapes=[
            pltpu.VMEM((NSEG, D, L), bf16),
            pltpu.VMEM((D, D), bf16),
            pltpu.VMEM((D, D), bf16),
            pltpu.VMEM((D, D), bf16),
            pltpu.VMEM((D, D), bf16),
            pltpu.VMEM((NT, 192, D), u32),
            pltpu.VMEM((D // 2, DP), u32),
            pltpu.VMEM((8, DP), f32),
            pltpu.VMEM((H + G, 8, 128), f32),
            pltpu.VMEM((2, D // 2, 128), f32),
            pltpu.VMEM((D // 2, L), u32),
            pltpu.VMEM((NT, 64, L), u32),
            pltpu.VMEM((NT, L // 2, 128), u32),
            pltpu.VMEM((DP // 2, L), u32),
            pltpu.VMEM((NT, 64, L), u32),
            pltpu.VMEM((NT, 64, L), u32),
            pltpu.VMEM((DP, L), f32),
            pltpu.VMEM((H + G, 32, L), f32),
            pltpu.VMEM((G, 128, 128), f32),
            pltpu.VMEM((G, 256, 128), f32),
            pltpu.VMEM((G, 384, 128), f32),
            pltpu.VMEM((G, 512, 128), f32),
            pltpu.VMEM((4, G, 8, 128), f32),
            pltpu.VMEM((G, 32, 128), f32),
            pltpu.VMEM((NT, 128, 128), f32),
            *[pltpu.VMEM((DP // 2, 128), u32)] * 2,
            *[pltpu.VMEM((D // 2, 128), u32)] * 4,
            pltpu.VMEM((S // 128, D // 2, 128), u32),
            pltpu.VMEM((S // 128, D // 2, 128), u32),
            pltpu.VMEM((NSEG, 8, L), f32),
            pltpu.VMEM((NSEG, D, L), bf16),
            pltpu.VMEM((D, 128), bf16),
            pltpu.VMEM((D, F), bf16),
            pltpu.VMEM((D, F), bf16),
            pltpu.VMEM((D, F), bf16),
            pltpu.SMEM((4,), jnp.int32),
            pltpu.SemaphoreType.DMA((3 + NSEG,)),
            pltpu.SemaphoreType.DMA((3 * NT + 1,)),
            pltpu.SemaphoreType.DMA((3,)),
            pltpu.SemaphoreType.DMA((NSEG + 1,)),
        ],
        compiler_params=pltpu.CompilerParams(vmem_limit_bytes=100 * 1024 * 1024),
    )(A_x.reshape(S, D).T, A_wq, A_wk, A_wv, A_wo, A_beta, B_w_r,
      B_w_gate, B_w_up, B_w_down.T)
    return out_t.T.reshape(1, S, D)
```

```python
import numpy as np
import jax
import jax.numpy as jnp
from jax import lax
import jax.experimental.pallas as pl
import jax.experimental.pallas.tpu as pltpu

S, D, H, DH = 2048, 576, 32, 18
NSEG, L = 4, 512
F = 4608
HPT = 7
NT = 5
DP = NT * 128
LOG2E = float(np.log2(np.e))
QSCALE = float(DH ** -0.5) * LOG2E
EPS_BF16 = float(np.asarray(1e-5, dtype=jnp.bfloat16).astype(np.float32))

bf16 = jnp.bfloat16
f32 = jnp.float32
u32 = jnp.uint32
G = 4
LAG = 5
STEPS = [(j, i) for j in range(4) for i in range(j + 1)]
NT_DIMS = (((1,), (1,)), ((), ()))


def _rb(x):
    return x.astype(bf16).astype(f32)


def _pack(x):
    return pltpu.bitcast(x, u32)


def _unpack(x):
    return pltpu.bitcast(x, bf16)


def _split(u):
    return tuple(pltpu.unpack_elementwise(u, index=i, packed_dtype=bf16, unpacked_dtype=f32)
                 for i in range(2))


def _merge(even, odd):
    return pltpu.pack_elementwise([even, odd], packed_dtype=bf16)


def _eo(x):
    n, m = x.shape[0] // 16, x.shape[1]
    x = x.reshape(n, 2, 8, m)
    return x[:, 0].reshape(8 * n, m), x[:, 1].reshape(8 * n, m)


def _eo_rows(u):
    n, m = u.shape[0] // 8, u.shape[1]
    even, odd = _split(u)
    x = jnp.concatenate([even.reshape(n, 8, m), odd.reshape(n, 8, m)], axis=1)
    return _pack(x.reshape(16 * n, m).astype(bf16))


def _pair_rows(u):
    n, m = u.shape[0] // 8, u.shape[1]
    x = _unpack(u).astype(f32).reshape(n, 2, 8, m)
    return _merge(x[:, 0].reshape(8 * n, m), x[:, 1].reshape(8 * n, m))


def _tree(op, x):
    parts = [x[8 * i:8 * (i + 1)] for i in range(x.shape[0] // 8)]
    while len(parts) > 1:
        parts = [op(parts[i], parts[i + 1]) if i + 1 < len(parts) else parts[i]
                 for i in range(0, len(parts), 2)]
    return parts[0]


def _colsum(pairs):
    part = jnp.concatenate([_tree(jnp.add, x) for pair in pairs for x in pair], axis=0)
    return jnp.sum(_tree(jnp.add, part), axis=0, keepdims=True)


def _head_rows(blocks):
    prev = None
    for t in range(NT):
        cur = blocks(t)
        tile = cur if t == 0 else jnp.concatenate([prev[64 - t:], cur[:64 - t]], axis=0)
        valid = min(HPT * DH, D - HPT * DH * t) // 2
        row = lax.broadcasted_iota(jnp.int32, tile.shape, 0)
        yield jnp.where(row < valid, tile, jnp.uint32(0))
        prev = cur


def _col_block_t(w_ref, i):
    if 128 * (i + 1) <= D:
        c = w_ref[:, 128 * i:128 * (i + 1)]
    else:
        c = jnp.concatenate([w_ref[:, 128 * i:], jnp.zeros((D, 128 * (i + 1) - D), bf16)], axis=1)
    return _pack(c.T)


def _row_block(w_ref, i):
    if 128 * (i + 1) <= D:
        return _pack(w_ref[128 * i:128 * (i + 1), :])
    r = _pack(w_ref[128 * i:, :])
    return jnp.concatenate([r, jnp.zeros((64 - r.shape[0], D), u32)], axis=0)


def _interleave(*gens):
    gens = list(gens)
    while gens:
        for g in list(gens):
            try:
                next(g)
            except StopIteration:
                gens.remove(g)


def _phi(t):
    return jnp.where(t > 0, t + 1.0, jnp.exp(t))


def _kernel(xt_hbm, wq_hbm, wk_hbm, wv_hbm, wo_hbm, beta_ref, wr_ref, wg_hbm, wu_hbm, wdt_hbm,
            o_hbm,
            xt_s, wq_s, wk_s, wv_s, wo_s, wc_s, wot_s, gl_s, g1_s, wr_s,
            lnt_s, q_s, k_s, vt_s, pq_s, pk_s, am_s, ow_s, s0_s, s1_s, s2_s, s3_s, mx_s,
            m_s, ob0_s, ob1_s, h0_s, h1_s, h2_s, h3_s, h_s, hn_s, r_s, out_s, patch_s,
            wg_s, wu_s, wdt_s, zero_s, sem_x, sem_w, sem_f, sem_o):
    def cols(i):
        return slice(128 * i, min(128 * (i + 1), D))

    x0_cp = [pltpu.make_async_copy(xt_hbm.at[:, cols(j)], xt_s.at[0, :, cols(j)], sem_x.at[j])
             for j in range(4)]
    x_cp = [None] + [pltpu.make_async_copy(xt_hbm.at[:, s * L:(s + 1) * L], xt_s.at[s],
                                           sem_x.at[3 + s]) for s in range(1, NSEG)]
    w_cp = [[pltpu.make_async_copy(src.at[:, cols(i)], dst.at[:, cols(i)], sem_w.at[3 * i + n])
             for n, (src, dst) in enumerate([(wq_hbm, wq_s), (wk_hbm, wk_s), (wv_hbm, wv_s)])]
            for i in range(NT)]
    wo_cp = pltpu.make_async_copy(wo_hbm, wo_s, sem_w.at[3 * NT])
    f_cp = [pltpu.make_async_copy(src, dst, sem_f.at[i]) for i, (src, dst) in enumerate(
        [(wg_hbm, wg_s), (wu_hbm, wu_s), (wdt_hbm, wdt_s)])]
    for c in x0_cp + w_cp[0]:
        c.start()
    for i in range(1, NT):
        for c in w_cp[i]:
            c.start()
    wo_cp.start()

    for k in range(4):
        zero_s[k] = 0
    g = _rb(jax.nn.sigmoid(beta_ref[...].astype(f32).reshape(1, H)))
    hrow = lax.broadcasted_iota(jnp.int32, (H, DP), 0)
    fcol = lax.broadcasted_iota(jnp.int32, (H, DP), 1)
    expand = ((fcol % 128) // DH + (fcol // 128) * HPT == hrow) & (fcol % 128 < HPT * DH)
    gl_s[...] = jnp.dot(jnp.broadcast_to(g, (16, H)).astype(bf16), expand.astype(bf16),
                        preferred_element_type=f32)[0:8]
    pick = (lax.broadcasted_iota(jnp.int32, (H * 8, H), 0) // 8
            == lax.broadcasted_iota(jnp.int32, (H * 8, H), 1))
    g1_s[...] = lax.dot_general(pick.astype(bf16),
                                jnp.broadcast_to(_rb(1.0 - g), (128, H)).astype(bf16), NT_DIMS,
                                preferred_element_type=f32).reshape(H, 8, 128)
    wr_rows = jnp.broadcast_to(wr_ref[...].reshape(1, D), (128, D)).T
    wr_s[0], wr_s[1] = _split(_pack(wr_rows))
    m_s[...] = jnp.zeros(m_s.shape, f32)

    def ln_steps(load, store):
        def chunks(k):
            return [_split(load(pl.multiple_of(zero_s[k] + 72 * c, 8)))
                    for c in range(4)]

        m = _colsum(chunks(0)) * (1.0 / D)
        yield
        sq = []
        for x in chunks(1):
            c = (x[0] - m, x[1] - m)
            sq.append((c[0] * c[0], c[1] * c[1]))
        v = _colsum(sq) * (1.0 / D)
        inv = 1.0 / _rb(jnp.sqrt(_rb(_rb(v) + EPS_BF16)))
        off = m * inv
        yield
        for c, x in enumerate(chunks(2)):
            store(72 * c, 72 * (c + 1), x, (x[0] * inv - off, x[1] * inv - off))
            if c % 2 == 1:
                yield

    def ln1_tile(s, j):
        cs = slice(128 * j, 128 * (j + 1))

        def store(lo, hi, x, y):
            lnt_s[lo:hi, cs] = _merge(*y)
        return ln_steps(
            lambda lo: _pack(xt_s[s, pl.ds(pl.multiple_of(2 * lo, 16), 144), cs]), store)

    s_refs = [s0_s, s1_s, s2_s, s3_s]
    ob_tiles = [ob0_s, ob1_s]
    h_tiles = [h0_s, h1_s, h2_s, h3_s]

    def qk_step(g, j, i, qs, mx):
        for a in range(G):
            t, r = divmod(G * g + a, HPT)
            if i == 0:
                row = lax.broadcasted_iota(jnp.int32, (64, 128), 0)
                head_rows = (row >= (DH // 2) * r) & (row < (DH // 2) * (r + 1))
                qs[a] = _unpack(jnp.where(head_rows, q_s[t, :, 128 * j:128 * (j + 1)],
                                          jnp.uint32(0)))
            kk = _unpack(k_s[t, 64 * i:64 * (i + 1), :])
            st = jnp.dot(kk, qs[a], preferred_element_type=f32)
            if i == j:
                krow = lax.broadcasted_iota(jnp.int32, (128, 128), 0)
                qcol = lax.broadcasted_iota(jnp.int32, (128, 128), 1)
                st = jnp.where(krow <= qcol, st, -1e30)
            s_refs[j][a, 128 * i:128 * (i + 1), :] = st
            m8 = _tree(jnp.maximum, st)
            mx[a] = m8 if i == 0 else jnp.maximum(mx[a], m8)
            if i == j:
                mx_s[j, a] = jnp.broadcast_to(jnp.max(mx[a], axis=0, keepdims=True), (8, 128))

    def sm_step(g, j, i, acc):
        for a in range(G):
            h = G * g + a
            base = 64 * (h // HPT) + 8 * (h % HPT)
            st = s_refs[j][a, 128 * i:128 * (i + 1), :]
            m = mx_s[j, a]
            p = jnp.exp2(st.reshape(16, 8, 128) - m[None]).reshape(128, 128).astype(bf16)
            vw = vt_s[base:base + 16, 128 * i:128 * (i + 1)]
            vw = jnp.where(lax.broadcasted_iota(jnp.int32, (16, 128), 0) == 15,
                           jnp.uint32(0x3F803F80), vw)
            d = jnp.dot(_unpack(vw), p, preferred_element_type=f32)
            acc[a] = d if i == 0 else acc[a] + d
            if i == j:
                scale = g1_s[h] / acc[a][24:32]
                ow_s[h, :, 128 * j:128 * (j + 1)] = acc[a] * scale[6:7]

    steps = [(g, j, i) for g in range(H // G) for (j, i) in STEPS]

    def attention():
        qs, mx, acc = [None] * G, [None] * G, [None] * G
        for n, step in enumerate(steps):
            qk_step(*step, qs, mx)
            if n >= LAG:
                sm_step(*steps[n - LAG], acc)

        def tail():
            for step in steps[len(steps) - LAG:]:
                sm_step(*step, acc)
                yield
        return tail()

    def project(t):
        rows = 64 if t < NT - 1 else 40
        w = wc_s[t]
        w = jnp.concatenate([w[0:rows], w[64:64 + rows], w[128:128 + rows]], axis=0)
        qkv = jnp.dot(_unpack(w), _unpack(lnt_s[...]), preferred_element_type=f32)
        n = 2 * rows

        def full(u):
            return u if rows == 64 else jnp.concatenate(
                [u, jnp.zeros((64 - rows, L), u32)], axis=0)

        qf, kf, vf = _eo(qkv[0:n]), _eo(qkv[n:2 * n]), _eo(qkv[2 * n:3 * n])
        q_s[t] = full(_merge(qf[0] * QSCALE, qf[1] * QSCALE))
        k_s[t] = _pack(_unpack(full(_merge(*kf))).T)
        vt = full(_merge(*vf))
        vt_s[64 * t:64 * (t + 1), :] = vt
        pq_s[t] = full(_merge(_phi(qf[0]), _phi(qf[1])))
        pk_s[t] = full(_merge(_phi(kf[0]), _phi(kf[1])))

    def memory_read(t):
        erow = lax.broadcasted_iota(jnp.int32, (128, 128), 0)
        dcol = lax.broadcasted_iota(jnp.int32, (128, 128), 1)
        bd_mask = (erow // DH == dcol // DH) & (dcol < HPT * DH)
        zrow = lax.broadcasted_iota(jnp.int32, (16, 128), 0)
        zcol = lax.broadcasted_iota(jnp.int32, (16, 128), 1)
        z_mask = (zcol // DH == zrow) & (zcol < HPT * DH)
        mt = m_s[t]
        pq = _unpack(pq_s[t])
        mb = jnp.where(bd_mask, mt * gl_s[0:1, 128 * t:128 * (t + 1)], 0.0)
        zb = jnp.where(z_mask, jnp.broadcast_to(mt[126:127, :], (16, 128)), 0.0)
        nd = jnp.dot(jnp.concatenate([mb, zb], axis=0).astype(bf16), pq,
                     preferred_element_type=f32)
        inv = 1.0 / (nd[128:136] + 1e-6)
        row8 = lax.broadcasted_iota(jnp.int32, (8, L), 0)
        bro = [jnp.broadcast_to(inv[a:a + 1], (8, L)) for a in range(HPT)]
        for u in range(16):
            ha, hb = (8 * u) // DH, min((8 * u + 7) // DH, HPT - 1)
            sc = bro[ha] if ha == hb else jnp.where(row8 < DH * hb - 8 * u, bro[ha], bro[hb])
            am_s[128 * t + 8 * u:128 * t + 8 * (u + 1), :] = nd[8 * u:8 * (u + 1)] * sc

    def memory_update(t):
        vone = jnp.where(lax.broadcasted_iota(jnp.int32, (64, L), 0) == 63,
                         jnp.uint32(0x3F803F80), vt_s[64 * t:64 * (t + 1), :])
        m_s[t] += lax.dot_general(_unpack(vone), _unpack(pk_s[t]), NT_DIMS,
                                  preferred_element_type=f32)

    def mix_tile(j):
        cs = slice(128 * j, 128 * (j + 1))
        row8 = lax.broadcasted_iota(jnp.int32, (8, 128), 0)
        parts = []
        for t in range(NT):
            for u in range(16):
                rr, half = u // 2, u % 2
                h = HPT * t + rr
                cut = 2 * rr - 8 * half
                lo_ok, hi_ok = (rr > 0 and h - 1 < H), (rr < HPT and h < H)
                lo = ow_s[h - 1, 16 + 8 * half:24 + 8 * half, cs] if lo_ok else None
                hi = ow_s[h, 8 * half:8 * half + 8, cs] if hi_ok else None
                if cut <= 0 or not lo_ok:
                    dp = hi
                elif cut >= 8 or not hi_ok:
                    dp = lo
                else:
                    dp = jnp.where(row8 >= cut, hi, lo)
                am = am_s[128 * t + 8 * u:128 * t + 8 * (u + 1), cs]
                parts.append(am if dp is None else am + dp)
            ob_tiles[j % 2][64 * t:64 * (t + 1), :] = _merge(
                jnp.concatenate(parts[0::2], axis=0), jnp.concatenate(parts[1::2], axis=0))
            parts = []
            if t % 2 == 1:
                yield
        yield

    def out_proj_tile(s, j):
        cs = slice(128 * j, 128 * (j + 1))
        for c in range(4):
            w = _unpack(wot_s[72 * c:72 * (c + 1), :])
            attn = _eo(jnp.dot(w, _unpack(ob_tiles[j % 2][...]), preferred_element_type=f32))
            x = _split(_pack(xt_s[s, 144 * c:144 * (c + 1), cs]))
            hb = _merge(x[0] + attn[0], x[1] + attn[1])
            h_tiles[j][72 * c:72 * (c + 1), :] = hb
            h_s[4 * s + j, 72 * c:72 * (c + 1), :] = hb
            yield

    def ln2_tile(s, j):
        cs = slice(128 * j, 128 * (j + 1))
        score = []

        def store(lo, hi, h, hn):
            out_s[s, 2 * lo:2 * hi, cs] = _unpack(_merge(h[0] + hn[0], h[1] + hn[1]))
            hn_s[4 * s + j, lo:hi, :] = _merge(*hn)
            score.append(_tree(jnp.add, hn[0] * wr_s[0, lo:hi])
                         + _tree(jnp.add, hn[1] * wr_s[1, lo:hi]))
            if hi == D // 2:
                r_s[s, :, cs] = (score[0] + score[1]) + (score[2] + score[3])
        return ln_steps(lambda lo: h_tiles[j][pl.ds(lo, 72), :], store)

    wq_t = _head_rows(lambda i: _col_block_t(wq_s, i))
    wk_t = _head_rows(lambda i: _col_block_t(wk_s, i))
    wv_t = _head_rows(lambda i: _col_block_t(wv_s, i))
    wo_t = _head_rows(lambda i: _row_block(wo_s, i))

    def first_weights():
        for rows, tiles in ((0, wq_t), (64, wk_t), (128, wv_t)):
            wc_s[0, rows:rows + 64, :] = _eo_rows(next(tiles))
            yield

    def first_ln(j):
        x0_cp[j].wait()
        yield from ln1_tile(0, j)

    for j in range(4):
        _interleave(first_ln(j))
    for c in w_cp[0]:
        c.wait()
    _interleave(first_weights())
    for c in [c for i in range(1, NT) for c in w_cp[i]] + [wo_cp]:
        c.wait()
    for c in x_cp[1:] + f_cp:
        c.start()
    for t in range(NT):
        if t + 1 < NT:
            wc_s[t + 1] = jnp.concatenate(
                [_eo_rows(next(wq_t)), _eo_rows(next(wk_t)), _eo_rows(next(wv_t))], axis=0)
        project(t)
        wot_s[:, 128 * t:128 * (t + 1)] = _eo_rows(_pack(_unpack(_pair_rows(next(wo_t))).T))

    def segment(s, last):
        if not last:
            pltpu.make_async_copy(xt_s.at[s + 1], xt_s.at[s + 1], sem_x.at[4 + s]).wait()

        tail = attention()

        def reads():
            for t in range(NT):
                memory_read(t)
                yield

        def updates():
            for t in range(NT):
                memory_update(t)
                yield

        _interleave(reads(), tail)
        _interleave(mix_tile(0), *([] if last else [updates()]))
        for j in range(4):
            gens = [out_proj_tile(s, j)]
            if not last:
                gens.append(ln1_tile(s + 1, j))
            if j < 3:
                gens.append(mix_tile(j + 1))
            if j > 0:
                gens.append(ln2_tile(s, j - 1))
            _interleave(*gens)

        def finish():
            yield from ln2_tile(s, 3)
            lo = s * L if last else pl.multiple_of(s * L, L)
            pltpu.make_async_copy(out_s.at[s], o_hbm.at[:, pl.ds(lo, L)], sem_o.at[s]).start()

        def next_projections():
            for t in range(NT):
                project(t)
                yield

        if last:
            _interleave(finish())
        else:
            _interleave(next_projections(), finish())

    def segment_body(s, carry):
        segment(s, False)
        return carry

    lax.fori_loop(0, NSEG - 1, segment_body, 0)
    segment(NSEG - 1, True)

    rall = jnp.concatenate([_rb(jnp.sum(r_s[s], axis=0, keepdims=True))
                            for s in range(NSEG)], axis=0)
    rmax = jnp.max(rall)
    pos = (lax.broadcasted_iota(jnp.int32, (NSEG, L), 0) * L
           + lax.broadcasted_iota(jnp.int32, (NSEG, L), 1))
    idx = jnp.clip(jnp.min(jnp.where(rall == rmax, pos, S)), 0, S - 1)
    tt = idx // 128
    ln_sel = idx - tt * 128
    rsel = _rb(jax.nn.sigmoid(jnp.full((1, 1), rmax, f32)))
    hn_t = _unpack(hn_s[tt])
    h_t = _unpack(h_s[tt]).astype(f32)
    onehot = (lax.broadcasted_iota(jnp.int32, (16, 128), 1) == ln_sel).astype(bf16)
    xsel = lax.dot_general(onehot, hn_t, NT_DIMS, preferred_element_type=f32).astype(bf16)

    f_cp[0].wait()
    f_cp[1].wait()
    gate = _rb(jnp.dot(xsel, wg_s[...], preferred_element_type=f32))
    up = _rb(jnp.dot(xsel, wu_s[...], preferred_element_type=f32))
    gu = (_rb(gate * jax.nn.sigmoid(gate)) * up).astype(bf16)
    f_cp[2].wait()
    y = _rb(lax.dot_general(gu, wdt_s[...], NT_DIMS, preferred_element_type=f32))
    y = _rb(y * rsel)
    yt = jnp.broadcast_to(y[0:1], (128, D)).T
    upd = jnp.where(lax.broadcasted_iota(jnp.int32, (D, 128), 1) == ln_sel, yt, 0.0)
    patch_s[...] = (h_t + _rb(hn_t.astype(f32) + upd)).astype(bf16)
    for s in range(NSEG):
        pltpu.make_async_copy(out_s.at[s], o_hbm.at[:, s * L:(s + 1) * L], sem_o.at[s]).wait()
    cp = pltpu.make_async_copy(patch_s, o_hbm.at[:, pl.ds(pl.multiple_of(tt * 128, 128), 128)],
                               sem_o.at[NSEG])
    cp.start()
    cp.wait()


@jax.jit
def pallas_sequential_preLN__memory_aug_infini_attn__moe_arch_mod__prompt_kernel(
    A_x: jax.Array,
    A_wq: jax.Array,
    A_wk: jax.Array,
    A_wv: jax.Array,
    A_wo: jax.Array,
    A_beta: jax.Array,
    B_x: jax.Array,
    B_w_r: jax.Array,
    B_w_gate: jax.Array,
    B_w_up: jax.Array,
    B_w_down: jax.Array,
):
    del B_x
    vmem = pl.BlockSpec(memory_space=pltpu.VMEM)
    hbm = pl.BlockSpec(memory_space=pltpu.HBM)
    out_t = pl.pallas_call(
        _kernel,
        out_shape=jax.ShapeDtypeStruct((D, S), bf16),
        in_specs=[hbm, hbm, hbm, hbm, hbm, vmem, vmem, hbm, hbm, hbm],
        out_specs=hbm,
        scratch_shapes=[
            pltpu.VMEM((NSEG, D, L), bf16),
            pltpu.VMEM((D, D), bf16),
            pltpu.VMEM((D, D), bf16),
            pltpu.VMEM((D, D), bf16),
            pltpu.VMEM((D, D), bf16),
            pltpu.VMEM((NT, 192, D), u32),
            pltpu.VMEM((D // 2, DP), u32),
            pltpu.VMEM((8, DP), f32),
            pltpu.VMEM((H, 8, 128), f32),
            pltpu.VMEM((2, D // 2, 128), f32),
            pltpu.VMEM((D // 2, L), u32),
            pltpu.VMEM((NT, 64, L), u32),
            pltpu.VMEM((NT, L // 2, 128), u32),
            pltpu.VMEM((DP // 2, L), u32),
            pltpu.VMEM((NT, 64, L), u32),
            pltpu.VMEM((NT, 64, L), u32),
            pltpu.VMEM((DP, L), f32),
            pltpu.VMEM((H, 32, L), f32),
            pltpu.VMEM((G, 128, 128), f32),
            pltpu.VMEM((G, 256, 128), f32),
            pltpu.VMEM((G, 384, 128), f32),
            pltpu.VMEM((G, 512, 128), f32),
            pltpu.VMEM((4, G, 8, 128), f32),
            pltpu.VMEM((NT, 128, 128), f32),
            *[pltpu.VMEM((DP // 2, 128), u32)] * 2,
            *[pltpu.VMEM((D // 2, 128), u32)] * 4,
            pltpu.VMEM((S // 128, D // 2, 128), u32),
            pltpu.VMEM((S // 128, D // 2, 128), u32),
            pltpu.VMEM((NSEG, 8, L), f32),
            pltpu.VMEM((NSEG, D, L), bf16),
            pltpu.VMEM((D, 128), bf16),
            pltpu.VMEM((D, F), bf16),
            pltpu.VMEM((D, F), bf16),
            pltpu.VMEM((D, F), bf16),
            pltpu.SMEM((4,), jnp.int32),
            pltpu.SemaphoreType.DMA((3 + NSEG,)),
            pltpu.SemaphoreType.DMA((3 * NT + 1,)),
            pltpu.SemaphoreType.DMA((3,)),
            pltpu.SemaphoreType.DMA((NSEG + 1,)),
        ],
        compiler_params=pltpu.CompilerParams(vmem_limit_bytes=100 * 1024 * 1024),
    )(A_x.reshape(S, D).T, A_wq, A_wk, A_wv, A_wo, A_beta, B_w_r,
      B_w_gate, B_w_up, B_w_down.T)
    return out_t.T.reshape(1, S, D)
```

```python
import numpy as np
import jax
import jax.numpy as jnp
from jax import lax
import jax.experimental.pallas as pl
import jax.experimental.pallas.tpu as pltpu

S, D, H, DH = 2048, 576, 32, 18
NSEG, L = 4, 512
F = 4608
HPT = 7
NT = 5
DP = NT * 128
LOG2E = float(np.log2(np.e))
QSCALE = float(DH ** -0.5) * LOG2E
EPS_BF16 = float(np.asarray(1e-5, dtype=jnp.bfloat16).astype(np.float32))

bf16 = jnp.bfloat16
f32 = jnp.float32
u32 = jnp.uint32
G = 4
LAG = 5
STEPS = [(j, i) for j in range(4) for i in range(j + 1)]
NT_DIMS = (((1,), (1,)), ((), ()))


def _rb(x):
    return x.astype(bf16).astype(f32)


def _pack(x):
    return pltpu.bitcast(x, u32)


def _unpack(x):
    return pltpu.bitcast(x, bf16)


def _split(u):
    return tuple(pltpu.unpack_elementwise(u, index=i, packed_dtype=bf16, unpacked_dtype=f32)
                 for i in range(2))


def _merge(even, odd):
    return pltpu.pack_elementwise([even, odd], packed_dtype=bf16)


def _eo(x):
    n, m = x.shape[0] // 16, x.shape[1]
    x = x.reshape(n, 2, 8, m)
    return x[:, 0].reshape(8 * n, m), x[:, 1].reshape(8 * n, m)


def _eo_rows(u):
    n, m = u.shape[0] // 8, u.shape[1]
    even, odd = _split(u)
    x = jnp.concatenate([even.reshape(n, 8, m), odd.reshape(n, 8, m)], axis=1)
    return _pack(x.reshape(16 * n, m).astype(bf16))


def _pair_rows(u):
    n, m = u.shape[0] // 8, u.shape[1]
    x = _unpack(u).astype(f32).reshape(n, 2, 8, m)
    return _merge(x[:, 0].reshape(8 * n, m), x[:, 1].reshape(8 * n, m))


def _tree(op, x):
    parts = [x[8 * i:8 * (i + 1)] for i in range(x.shape[0] // 8)]
    while len(parts) > 1:
        parts = [op(parts[i], parts[i + 1]) if i + 1 < len(parts) else parts[i]
                 for i in range(0, len(parts), 2)]
    return parts[0]


def _colsum(pairs):
    part = jnp.concatenate([_tree(jnp.add, x) for pair in pairs for x in pair], axis=0)
    return jnp.sum(_tree(jnp.add, part), axis=0, keepdims=True)


def _head_rows(blocks):
    prev = None
    for t in range(NT):
        cur = blocks(t)
        tile = cur if t == 0 else jnp.concatenate([prev[64 - t:], cur[:64 - t]], axis=0)
        valid = min(HPT * DH, D - HPT * DH * t) // 2
        row = lax.broadcasted_iota(jnp.int32, tile.shape, 0)
        yield jnp.where(row < valid, tile, jnp.uint32(0))
        prev = cur


def _col_block_t(w_ref, i):
    if 128 * (i + 1) <= D:
        c = w_ref[:, 128 * i:128 * (i + 1)]
    else:
        c = jnp.concatenate([w_ref[:, 128 * i:], jnp.zeros((D, 128 * (i + 1) - D), bf16)], axis=1)
    return _pack(c.T)


def _row_block(w_ref, i):
    if 128 * (i + 1) <= D:
        return _pack(w_ref[128 * i:128 * (i + 1), :])
    r = _pack(w_ref[128 * i:, :])
    return jnp.concatenate([r, jnp.zeros((64 - r.shape[0], D), u32)], axis=0)


def _interleave(*gens):
    gens = list(gens)
    while gens:
        for g in list(gens):
            try:
                next(g)
            except StopIteration:
                gens.remove(g)


def _phi(t):
    return jnp.where(t > 0, t + 1.0, jnp.exp(t))


def _kernel(xt_hbm, wq_hbm, wk_hbm, wv_hbm, wo_hbm, beta_ref, wr_ref, wg_hbm, wu_hbm, wdt_hbm,
            o_hbm,
            xt_s, wq_s, wk_s, wv_s, wo_s, wc_s, wot_s, gl_s, g1_s, wr_s,
            lnt_s, q_s, k_s, vt_s, pq_s, pk_s, am_s, ow_s, s0_s, s1_s, s2_s, s3_s, mx_s,
            m_s, ob0_s, ob1_s, h0_s, h1_s, h2_s, h3_s, h_s, hn_s, r_s, out_s, patch_s,
            wg_s, wu_s, wdt_s, zero_s, sem_x, sem_w, sem_f, sem_o):
    def cols(i):
        return slice(128 * i, min(128 * (i + 1), D))

    x0_cp = [pltpu.make_async_copy(xt_hbm.at[:, cols(j)], xt_s.at[0, :, cols(j)], sem_x.at[j])
             for j in range(4)]
    x_cp = [None] + [pltpu.make_async_copy(xt_hbm.at[:, s * L:(s + 1) * L], xt_s.at[s],
                                           sem_x.at[3 + s]) for s in range(1, NSEG)]
    w_cp = [[pltpu.make_async_copy(src.at[:, cols(i)], dst.at[:, cols(i)], sem_w.at[3 * i + n])
             for n, (src, dst) in enumerate([(wq_hbm, wq_s), (wk_hbm, wk_s), (wv_hbm, wv_s)])]
            for i in range(NT)]
    wo_cp = pltpu.make_async_copy(wo_hbm, wo_s, sem_w.at[3 * NT])
    f_cp = [pltpu.make_async_copy(src, dst, sem_f.at[i]) for i, (src, dst) in enumerate(
        [(wg_hbm, wg_s), (wu_hbm, wu_s), (wdt_hbm, wdt_s)])]
    for c in x0_cp + w_cp[0]:
        c.start()

    for k in range(4):
        zero_s[k] = 0
    g = _rb(jax.nn.sigmoid(beta_ref[...].astype(f32).reshape(1, H)))
    hrow = lax.broadcasted_iota(jnp.int32, (H, DP), 0)
    fcol = lax.broadcasted_iota(jnp.int32, (H, DP), 1)
    expand = ((fcol % 128) // DH + (fcol // 128) * HPT == hrow) & (fcol % 128 < HPT * DH)
    gl_s[...] = jnp.dot(jnp.broadcast_to(g, (16, H)).astype(bf16), expand.astype(bf16),
                        preferred_element_type=f32)[0:8]
    pick = (lax.broadcasted_iota(jnp.int32, (H * 8, H), 0) // 8
            == lax.broadcasted_iota(jnp.int32, (H * 8, H), 1))
    g1_s[...] = lax.dot_general(pick.astype(bf16),
                                jnp.broadcast_to(_rb(1.0 - g), (128, H)).astype(bf16), NT_DIMS,
                                preferred_element_type=f32).reshape(H, 8, 128)
    wr_rows = jnp.broadcast_to(wr_ref[...].reshape(1, D), (128, D)).T
    wr_s[0], wr_s[1] = _split(_pack(wr_rows))
    m_s[...] = jnp.zeros(m_s.shape, f32)

    def ln_steps(load, store):
        def chunks(k):
            return [_split(load(pl.multiple_of(zero_s[k] + 72 * c, 8)))
                    for c in range(4)]

        m = _colsum(chunks(0)) * (1.0 / D)
        yield
        sq = []
        for x in chunks(1):
            c = (x[0] - m, x[1] - m)
            sq.append((c[0] * c[0], c[1] * c[1]))
        v = _colsum(sq) * (1.0 / D)
        inv = 1.0 / _rb(jnp.sqrt(_rb(_rb(v) + EPS_BF16)))
        off = m * inv
        yield
        for c, x in enumerate(chunks(2)):
            store(72 * c, 72 * (c + 1), x, (x[0] * inv - off, x[1] * inv - off))
            if c % 2 == 1:
                yield

    def ln1_tile(s, j):
        cs = slice(128 * j, 128 * (j + 1))

        def store(lo, hi, x, y):
            lnt_s[lo:hi, cs] = _merge(*y)
        return ln_steps(
            lambda lo: _pack(xt_s[s, pl.ds(pl.multiple_of(2 * lo, 16), 144), cs]), store)

    s_refs = [s0_s, s1_s, s2_s, s3_s]
    ob_tiles = [ob0_s, ob1_s]
    h_tiles = [h0_s, h1_s, h2_s, h3_s]

    def qk_step(g, j, i, qs, mx):
        for a in range(G):
            t, r = divmod(G * g + a, HPT)
            if i == 0:
                row = lax.broadcasted_iota(jnp.int32, (64, 128), 0)
                head_rows = (row >= (DH // 2) * r) & (row < (DH // 2) * (r + 1))
                qs[a] = _unpack(jnp.where(head_rows, q_s[t, :, 128 * j:128 * (j + 1)],
                                          jnp.uint32(0)))
            kk = _unpack(k_s[t, 64 * i:64 * (i + 1), :])
            st = jnp.dot(kk, qs[a], preferred_element_type=f32)
            if i == j:
                krow = lax.broadcasted_iota(jnp.int32, (128, 128), 0)
                qcol = lax.broadcasted_iota(jnp.int32, (128, 128), 1)
                st = jnp.where(krow <= qcol, st, -1e30)
            s_refs[j][a, 128 * i:128 * (i + 1), :] = st
            m8 = _tree(jnp.maximum, st)
            mx[a] = m8 if i == 0 else jnp.maximum(mx[a], m8)
            if i == j:
                mx_s[j, a] = jnp.broadcast_to(jnp.max(mx[a], axis=0, keepdims=True), (8, 128))

    def sm_step(g, j, i, acc):
        for a in range(G):
            h = G * g + a
            base = 64 * (h // HPT) + 8 * (h % HPT)
            st = s_refs[j][a, 128 * i:128 * (i + 1), :]
            m = mx_s[j, a]
            p = jnp.exp2(st.reshape(16, 8, 128) - m[None]).reshape(128, 128).astype(bf16)
            vw = vt_s[base:base + 16, 128 * i:128 * (i + 1)]
            vw = jnp.where(lax.broadcasted_iota(jnp.int32, (16, 128), 0) == 15,
                           jnp.uint32(0x3F803F80), vw)
            d = jnp.dot(_unpack(vw), p, preferred_element_type=f32)
            acc[a] = d if i == 0 else acc[a] + d
            if i == j:
                scale = g1_s[h] / acc[a][24:32]
                ow_s[h, :, 128 * j:128 * (j + 1)] = acc[a] * scale[6:7]

    steps = [(g, j, i) for g in range(H // G) for (j, i) in STEPS]

    def attention():
        qs, mx, acc = [None] * G, [None] * G, [None] * G
        for n, step in enumerate(steps):
            qk_step(*step, qs, mx)
            if n >= LAG:
                sm_step(*steps[n - LAG], acc)

        def tail():
            for step in steps[len(steps) - LAG:]:
                sm_step(*step, acc)
                yield
        return tail()

    def project(t):
        rows = 64 if t < NT - 1 else 40
        w = wc_s[t]
        w = jnp.concatenate([w[0:rows], w[64:64 + rows], w[128:128 + rows]], axis=0)
        qkv = jnp.dot(_unpack(w), _unpack(lnt_s[...]), preferred_element_type=f32)
        n = 2 * rows

        def full(u):
            return u if rows == 64 else jnp.concatenate(
                [u, jnp.zeros((64 - rows, L), u32)], axis=0)

        qf, kf, vf = _eo(qkv[0:n]), _eo(qkv[n:2 * n]), _eo(qkv[2 * n:3 * n])
        q_s[t] = full(_merge(qf[0] * QSCALE, qf[1] * QSCALE))
        k_s[t] = _pack(_unpack(full(_merge(*kf))).T)
        vt = full(_merge(*vf))
        vt_s[64 * t:64 * (t + 1), :] = vt
        pq_s[t] = full(_merge(_phi(qf[0]), _phi(qf[1])))
        pk_s[t] = full(_merge(_phi(kf[0]), _phi(kf[1])))

    def memory_read(t):
        erow = lax.broadcasted_iota(jnp.int32, (128, 128), 0)
        dcol = lax.broadcasted_iota(jnp.int32, (128, 128), 1)
        bd_mask = (erow // DH == dcol // DH) & (dcol < HPT * DH)
        zrow = lax.broadcasted_iota(jnp.int32, (16, 128), 0)
        zcol = lax.broadcasted_iota(jnp.int32, (16, 128), 1)
        z_mask = (zcol // DH == zrow) & (zcol < HPT * DH)
        mt = m_s[t]
        pq = _unpack(pq_s[t])
        mb = jnp.where(bd_mask, mt * gl_s[0:1, 128 * t:128 * (t + 1)], 0.0)
        zb = jnp.where(z_mask, jnp.broadcast_to(mt[126:127, :], (16, 128)), 0.0)
        nd = jnp.dot(jnp.concatenate([mb, zb], axis=0).astype(bf16), pq,
                     preferred_element_type=f32)
        inv = 1.0 / (nd[128:136] + 1e-6)
        row8 = lax.broadcasted_iota(jnp.int32, (8, L), 0)
        bro = [jnp.broadcast_to(inv[a:a + 1], (8, L)) for a in range(HPT)]
        for u in range(16):
            ha, hb = (8 * u) // DH, min((8 * u + 7) // DH, HPT - 1)
            sc = bro[ha] if ha == hb else jnp.where(row8 < DH * hb - 8 * u, bro[ha], bro[hb])
            am_s[128 * t + 8 * u:128 * t + 8 * (u + 1), :] = nd[8 * u:8 * (u + 1)] * sc

    def memory_update(t):
        vone = jnp.where(lax.broadcasted_iota(jnp.int32, (64, L), 0) == 63,
                         jnp.uint32(0x3F803F80), vt_s[64 * t:64 * (t + 1), :])
        m_s[t] += lax.dot_general(_unpack(vone), _unpack(pk_s[t]), NT_DIMS,
                                  preferred_element_type=f32)

    def mix_tile(j):
        cs = slice(128 * j, 128 * (j + 1))
        row8 = lax.broadcasted_iota(jnp.int32, (8, 128), 0)
        parts = []
        for t in range(NT):
            for u in range(16):
                rr, half = u // 2, u % 2
                h = HPT * t + rr
                cut = 2 * rr - 8 * half
                lo_ok, hi_ok = (rr > 0 and h - 1 < H), (rr < HPT and h < H)
                lo = ow_s[h - 1, 16 + 8 * half:24 + 8 * half, cs] if lo_ok else None
                hi = ow_s[h, 8 * half:8 * half + 8, cs] if hi_ok else None
                if cut <= 0 or not lo_ok:
                    dp = hi
                elif cut >= 8 or not hi_ok:
                    dp = lo
                else:
                    dp = jnp.where(row8 >= cut, hi, lo)
                am = am_s[128 * t + 8 * u:128 * t + 8 * (u + 1), cs]
                parts.append(am if dp is None else am + dp)
            ob_tiles[j % 2][64 * t:64 * (t + 1), :] = _merge(
                jnp.concatenate(parts[0::2], axis=0), jnp.concatenate(parts[1::2], axis=0))
            parts = []
            if t % 2 == 1:
                yield
        yield

    def out_proj_tile(s, j):
        cs = slice(128 * j, 128 * (j + 1))
        for c in range(4):
            w = _unpack(wot_s[72 * c:72 * (c + 1), :])
            attn = _eo(jnp.dot(w, _unpack(ob_tiles[j % 2][...]), preferred_element_type=f32))
            x = _split(_pack(xt_s[s, 144 * c:144 * (c + 1), cs]))
            hb = _merge(x[0] + attn[0], x[1] + attn[1])
            h_tiles[j][72 * c:72 * (c + 1), :] = hb
            h_s[4 * s + j, 72 * c:72 * (c + 1), :] = hb
            yield

    def ln2_tile(s, j):
        cs = slice(128 * j, 128 * (j + 1))
        score = []

        def store(lo, hi, h, hn):
            out_s[s, 2 * lo:2 * hi, cs] = _unpack(_merge(h[0] + hn[0], h[1] + hn[1]))
            hn_s[4 * s + j, lo:hi, :] = _merge(*hn)
            score.append(_tree(jnp.add, hn[0] * wr_s[0, lo:hi])
                         + _tree(jnp.add, hn[1] * wr_s[1, lo:hi]))
            if hi == D // 2:
                r_s[s, :, cs] = (score[0] + score[1]) + (score[2] + score[3])
        return ln_steps(lambda lo: h_tiles[j][pl.ds(lo, 72), :], store)

    wq_t = _head_rows(lambda i: _col_block_t(wq_s, i))
    wk_t = _head_rows(lambda i: _col_block_t(wk_s, i))
    wv_t = _head_rows(lambda i: _col_block_t(wv_s, i))
    wo_t = _head_rows(lambda i: _row_block(wo_s, i))

    def first_weights():
        for rows, tiles in ((0, wq_t), (64, wk_t), (128, wv_t)):
            wc_s[0, rows:rows + 64, :] = _eo_rows(next(tiles))
            yield

    def first_ln(j):
        x0_cp[j].wait()
        for c in w_cp[j + 1]:
            c.start()
        yield from ln1_tile(0, j)

    for j in range(4):
        _interleave(first_ln(j))
    def next_weights(t):
        wc_s[t] = jnp.concatenate(
            [_eo_rows(next(wq_t)), _eo_rows(next(wk_t)), _eo_rows(next(wv_t))], axis=0)

    def next_wo(t):
        wot_s[:, 128 * t:128 * (t + 1)] = _eo_rows(_pack(_unpack(_pair_rows(next(wo_t))).T))

    for c in w_cp[0]:
        c.wait()
    wo_cp.start()
    _interleave(first_weights())
    project(0)
    for c in w_cp[1] + w_cp[2]:
        c.wait()
    next_weights(1)
    next_weights(2)
    project(1)
    for c in w_cp[3] + w_cp[4] + [wo_cp]:
        c.wait()
    for c in x_cp[1:] + f_cp:
        c.start()
    for t in (2, 3, 4):
        if t < 4:
            next_weights(t + 1)
        project(t)
        for u in ((0,), (1, 2), (3, 4))[t - 2]:
            next_wo(u)

    def segment(s, last):
        if not last:
            pltpu.make_async_copy(xt_s.at[s + 1], xt_s.at[s + 1], sem_x.at[4 + s]).wait()

        tail = attention()

        def reads():
            for t in range(NT):
                memory_read(t)
                yield

        def updates():
            for t in range(NT):
                memory_update(t)
                yield

        _interleave(reads(), tail)
        _interleave(mix_tile(0), *([] if last else [updates()]))
        for j in range(4):
            gens = [out_proj_tile(s, j)]
            if not last:
                gens.append(ln1_tile(s + 1, j))
            if j < 3:
                gens.append(mix_tile(j + 1))
            if j > 0:
                gens.append(ln2_tile(s, j - 1))
            _interleave(*gens)

        def finish():
            yield from ln2_tile(s, 3)
            lo = s * L if last else pl.multiple_of(s * L, L)
            pltpu.make_async_copy(out_s.at[s], o_hbm.at[:, pl.ds(lo, L)], sem_o.at[s]).start()

        def next_projections():
            for t in range(NT):
                project(t)
                yield

        if last:
            _interleave(finish())
        else:
            _interleave(next_projections(), finish())

    def segment_body(s, carry):
        segment(s, False)
        return carry

    lax.fori_loop(0, NSEG - 1, segment_body, 0)
    segment(NSEG - 1, True)

    rall = jnp.concatenate([_rb(jnp.sum(r_s[s], axis=0, keepdims=True))
                            for s in range(NSEG)], axis=0)
    rmax = jnp.max(rall)
    pos = (lax.broadcasted_iota(jnp.int32, (NSEG, L), 0) * L
           + lax.broadcasted_iota(jnp.int32, (NSEG, L), 1))
    idx = jnp.clip(jnp.min(jnp.where(rall == rmax, pos, S)), 0, S - 1)
    tt = idx // 128
    ln_sel = idx - tt * 128
    rsel = _rb(jax.nn.sigmoid(jnp.full((1, 1), rmax, f32)))
    hn_t = _unpack(hn_s[tt])
    h_t = _unpack(h_s[tt]).astype(f32)
    onehot = (lax.broadcasted_iota(jnp.int32, (16, 128), 1) == ln_sel).astype(bf16)
    xsel = lax.dot_general(onehot, hn_t, NT_DIMS, preferred_element_type=f32).astype(bf16)

    f_cp[0].wait()
    f_cp[1].wait()
    gate = _rb(jnp.dot(xsel, wg_s[...], preferred_element_type=f32))
    up = _rb(jnp.dot(xsel, wu_s[...], preferred_element_type=f32))
    gu = (_rb(gate * jax.nn.sigmoid(gate)) * up).astype(bf16)
    f_cp[2].wait()
    y = _rb(lax.dot_general(gu, wdt_s[...], NT_DIMS, preferred_element_type=f32))
    y = _rb(y * rsel)
    yt = jnp.broadcast_to(y[0:1], (128, D)).T
    upd = jnp.where(lax.broadcasted_iota(jnp.int32, (D, 128), 1) == ln_sel, yt, 0.0)
    patch_s[...] = (h_t + _rb(hn_t.astype(f32) + upd)).astype(bf16)
    for s in range(NSEG):
        pltpu.make_async_copy(out_s.at[s], o_hbm.at[:, s * L:(s + 1) * L], sem_o.at[s]).wait()
    cp = pltpu.make_async_copy(patch_s, o_hbm.at[:, pl.ds(pl.multiple_of(tt * 128, 128), 128)],
                               sem_o.at[NSEG])
    cp.start()
    cp.wait()


@jax.jit
def pallas_sequential_preLN__memory_aug_infini_attn__moe_arch_mod__prompt_kernel(
    A_x: jax.Array,
    A_wq: jax.Array,
    A_wk: jax.Array,
    A_wv: jax.Array,
    A_wo: jax.Array,
    A_beta: jax.Array,
    B_x: jax.Array,
    B_w_r: jax.Array,
    B_w_gate: jax.Array,
    B_w_up: jax.Array,
    B_w_down: jax.Array,
):
    del B_x
    vmem = pl.BlockSpec(memory_space=pltpu.VMEM)
    hbm = pl.BlockSpec(memory_space=pltpu.HBM)
    out_t = pl.pallas_call(
        _kernel,
        out_shape=jax.ShapeDtypeStruct((D, S), bf16),
        in_specs=[hbm, hbm, hbm, hbm, hbm, vmem, vmem, hbm, hbm, hbm],
        out_specs=hbm,
        scratch_shapes=[
            pltpu.VMEM((NSEG, D, L), bf16),
            pltpu.VMEM((D, D), bf16),
            pltpu.VMEM((D, D), bf16),
            pltpu.VMEM((D, D), bf16),
            pltpu.VMEM((D, D), bf16),
            pltpu.VMEM((NT, 192, D), u32),
            pltpu.VMEM((D // 2, DP), u32),
            pltpu.VMEM((8, DP), f32),
            pltpu.VMEM((H, 8, 128), f32),
            pltpu.VMEM((2, D // 2, 128), f32),
            pltpu.VMEM((D // 2, L), u32),
            pltpu.VMEM((NT, 64, L), u32),
            pltpu.VMEM((NT, L // 2, 128), u32),
            pltpu.VMEM((DP // 2, L), u32),
            pltpu.VMEM((NT, 64, L), u32),
            pltpu.VMEM((NT, 64, L), u32),
            pltpu.VMEM((DP, L), f32),
            pltpu.VMEM((H, 32, L), f32),
            pltpu.VMEM((G, 128, 128), f32),
            pltpu.VMEM((G, 256, 128), f32),
            pltpu.VMEM((G, 384, 128), f32),
            pltpu.VMEM((G, 512, 128), f32),
            pltpu.VMEM((4, G, 8, 128), f32),
            pltpu.VMEM((NT, 128, 128), f32),
            *[pltpu.VMEM((DP // 2, 128), u32)] * 2,
            *[pltpu.VMEM((D // 2, 128), u32)] * 4,
            pltpu.VMEM((S // 128, D // 2, 128), u32),
            pltpu.VMEM((S // 128, D // 2, 128), u32),
            pltpu.VMEM((NSEG, 8, L), f32),
            pltpu.VMEM((NSEG, D, L), bf16),
            pltpu.VMEM((D, 128), bf16),
            pltpu.VMEM((D, F), bf16),
            pltpu.VMEM((D, F), bf16),
            pltpu.VMEM((D, F), bf16),
            pltpu.SMEM((4,), jnp.int32),
            pltpu.SemaphoreType.DMA((3 + NSEG,)),
            pltpu.SemaphoreType.DMA((3 * NT + 1,)),
            pltpu.SemaphoreType.DMA((3,)),
            pltpu.SemaphoreType.DMA((NSEG + 1,)),
        ],
        compiler_params=pltpu.CompilerParams(vmem_limit_bytes=100 * 1024 * 1024),
    )(A_x.reshape(S, D).T, A_wq, A_wk, A_wv, A_wo, A_beta, B_w_r,
      B_w_gate, B_w_up, B_w_down.T)
    return out_t.T.reshape(1, S, D)
```

```python
import numpy as np
import jax
import jax.numpy as jnp
from jax import lax
import jax.experimental.pallas as pl
import jax.experimental.pallas.tpu as pltpu

S, D, H, DH = 2048, 576, 32, 18
NSEG, L = 4, 512
F = 4608
FC = 512
HPT = 7
NT = 5
DP = NT * 128
LOG2E = float(np.log2(np.e))
QSCALE = float(DH ** -0.5) * LOG2E
EPS_BF16 = float(np.asarray(1e-5, dtype=jnp.bfloat16).astype(np.float32))

bf16 = jnp.bfloat16
f32 = jnp.float32
u32 = jnp.uint32
G = 4
LAG = 5
STEPS = [(j, i) for j in range(4) for i in range(j + 1)]
NT_DIMS = (((1,), (1,)), ((), ()))


def _rb(x):
    return x.astype(bf16).astype(f32)


def _pack(x):
    return pltpu.bitcast(x, u32)


def _unpack(x):
    return pltpu.bitcast(x, bf16)


def _split(u):
    return tuple(pltpu.unpack_elementwise(u, index=i, packed_dtype=bf16, unpacked_dtype=f32)
                 for i in range(2))


def _merge(even, odd):
    return pltpu.pack_elementwise([even, odd], packed_dtype=bf16)


def _eo(x):
    n, m = x.shape[0] // 16, x.shape[1]
    x = x.reshape(n, 2, 8, m)
    return x[:, 0].reshape(8 * n, m), x[:, 1].reshape(8 * n, m)


def _eo_rows(u):
    n, m = u.shape[0] // 8, u.shape[1]
    even, odd = _split(u)
    x = jnp.concatenate([even.reshape(n, 8, m), odd.reshape(n, 8, m)], axis=1)
    return _pack(x.reshape(16 * n, m).astype(bf16))


def _pair_rows(u):
    n, m = u.shape[0] // 8, u.shape[1]
    x = _unpack(u).astype(f32).reshape(n, 2, 8, m)
    return _merge(x[:, 0].reshape(8 * n, m), x[:, 1].reshape(8 * n, m))


def _tree(op, x):
    parts = [x[8 * i:8 * (i + 1)] for i in range(x.shape[0] // 8)]
    while len(parts) > 1:
        parts = [op(parts[i], parts[i + 1]) if i + 1 < len(parts) else parts[i]
                 for i in range(0, len(parts), 2)]
    return parts[0]


def _colsum(pairs):
    part = jnp.concatenate([_tree(jnp.add, x) for pair in pairs for x in pair], axis=0)
    return jnp.sum(_tree(jnp.add, part), axis=0, keepdims=True)


def _head_rows(blocks):
    prev = None
    for t in range(NT):
        cur = blocks(t)
        tile = cur if t == 0 else jnp.concatenate([prev[64 - t:], cur[:64 - t]], axis=0)
        valid = min(HPT * DH, D - HPT * DH * t) // 2
        row = lax.broadcasted_iota(jnp.int32, tile.shape, 0)
        yield jnp.where(row < valid, tile, jnp.uint32(0))
        prev = cur


def _col_block_t(w_ref, i):
    if 128 * (i + 1) <= D:
        c = w_ref[:, 128 * i:128 * (i + 1)]
    else:
        c = jnp.concatenate([w_ref[:, 128 * i:], jnp.zeros((D, 128 * (i + 1) - D), bf16)], axis=1)
    return _pack(c.T)


def _row_block(w_ref, i):
    if 128 * (i + 1) <= D:
        return _pack(w_ref[128 * i:128 * (i + 1), :])
    r = _pack(w_ref[128 * i:, :])
    return jnp.concatenate([r, jnp.zeros((64 - r.shape[0], D), u32)], axis=0)


def _interleave(*gens):
    gens = list(gens)
    while gens:
        for g in list(gens):
            try:
                next(g)
            except StopIteration:
                gens.remove(g)


def _phi(t):
    return jnp.where(t > 0, t + 1.0, jnp.exp(t))


def _kernel(xt_hbm, wq_hbm, wk_hbm, wv_hbm, wo_hbm, beta_ref, wr_ref, wg_hbm, wu_hbm, wdt_hbm,
            o_hbm,
            xt_s, wq_s, wk_s, wv_s, wo_s, wc_s, wot_s, gl_s, g1_s, wr_s,
            lnt_s, q_s, k_s, vt_s, pq_s, pk_s, am_s, ow_s, s0_s, s1_s, s2_s, s3_s, mx_s,
            m_s, ob0_s, ob1_s, h0_s, h1_s, h2_s, h3_s, h_s, hn_s, r_s, out_s, patch_s, ya_s,
            wg_s, wu_s, wdt_s, zero_s, sem_x, sem_w, sem_f, sem_o):
    def cols(i):
        return slice(128 * i, min(128 * (i + 1), D))

    x0_cp = [pltpu.make_async_copy(xt_hbm.at[:, cols(j)], xt_s.at[0, :, cols(j)], sem_x.at[j])
             for j in range(4)]
    x_cp = [None] + [pltpu.make_async_copy(xt_hbm.at[:, s * L:(s + 1) * L], xt_s.at[s],
                                           sem_x.at[3 + s]) for s in range(1, NSEG)]
    w_cp = [[pltpu.make_async_copy(src.at[:, cols(i)], dst.at[:, cols(i)], sem_w.at[3 * i + n])
             for n, (src, dst) in enumerate([(wq_hbm, wq_s), (wk_hbm, wk_s), (wv_hbm, wv_s)])]
            for i in range(NT)]
    wo_cp = pltpu.make_async_copy(wo_hbm, wo_s, sem_w.at[3 * NT])
    f_cp = [pltpu.make_async_copy(src, dst, sem_f.at[i]) for i, (src, dst) in enumerate(
        [(wg_hbm, wg_s), (wu_hbm, wu_s), (wdt_hbm, wdt_s)])]
    for c in x0_cp + w_cp[0]:
        c.start()

    for k in range(4):
        zero_s[k] = 0
    g = _rb(jax.nn.sigmoid(beta_ref[...].astype(f32).reshape(1, H)))
    hrow = lax.broadcasted_iota(jnp.int32, (H, DP), 0)
    fcol = lax.broadcasted_iota(jnp.int32, (H, DP), 1)
    expand = ((fcol % 128) // DH + (fcol // 128) * HPT == hrow) & (fcol % 128 < HPT * DH)
    gl_s[...] = jnp.dot(jnp.broadcast_to(g, (16, H)).astype(bf16), expand.astype(bf16),
                        preferred_element_type=f32)[0:8]
    pick = (lax.broadcasted_iota(jnp.int32, (H * 8, H), 0) // 8
            == lax.broadcasted_iota(jnp.int32, (H * 8, H), 1))
    g1_s[...] = lax.dot_general(pick.astype(bf16),
                                jnp.broadcast_to(_rb(1.0 - g), (128, H)).astype(bf16), NT_DIMS,
                                preferred_element_type=f32).reshape(H, 8, 128)
    wr_rows = jnp.broadcast_to(wr_ref[...].reshape(1, D), (128, D)).T
    wr_s[0], wr_s[1] = _split(_pack(wr_rows))
    m_s[...] = jnp.zeros(m_s.shape, f32)

    def ln_steps(load, store):
        def chunks(k):
            return [_split(load(pl.multiple_of(zero_s[k] + 72 * c, 8)))
                    for c in range(4)]

        m = _colsum(chunks(0)) * (1.0 / D)
        yield
        sq = []
        for x in chunks(1):
            c = (x[0] - m, x[1] - m)
            sq.append((c[0] * c[0], c[1] * c[1]))
        v = _colsum(sq) * (1.0 / D)
        inv = 1.0 / _rb(jnp.sqrt(_rb(_rb(v) + EPS_BF16)))
        off = m * inv
        yield
        for c, x in enumerate(chunks(2)):
            store(72 * c, 72 * (c + 1), x, (x[0] * inv - off, x[1] * inv - off))
            if c % 2 == 1:
                yield

    def ln1_tile(s, j):
        cs = slice(128 * j, 128 * (j + 1))

        def store(lo, hi, x, y):
            lnt_s[lo:hi, cs] = _merge(*y)
        return ln_steps(
            lambda lo: _pack(xt_s[s, pl.ds(pl.multiple_of(2 * lo, 16), 144), cs]), store)

    s_refs = [s0_s, s1_s, s2_s, s3_s]
    ob_tiles = [ob0_s, ob1_s]
    h_tiles = [h0_s, h1_s, h2_s, h3_s]

    def qk_step(g, j, i, qs, mx):
        for a in range(G):
            t, r = divmod(G * g + a, HPT)
            if i == 0:
                row = lax.broadcasted_iota(jnp.int32, (64, 128), 0)
                head_rows = (row >= (DH // 2) * r) & (row < (DH // 2) * (r + 1))
                qs[a] = _unpack(jnp.where(head_rows, q_s[t, :, 128 * j:128 * (j + 1)],
                                          jnp.uint32(0)))
            kk = _unpack(k_s[t, 64 * i:64 * (i + 1), :])
            st = jnp.dot(kk, qs[a], preferred_element_type=f32)
            if i == j:
                krow = lax.broadcasted_iota(jnp.int32, (128, 128), 0)
                qcol = lax.broadcasted_iota(jnp.int32, (128, 128), 1)
                st = jnp.where(krow <= qcol, st, -1e30)
            s_refs[j][a, 128 * i:128 * (i + 1), :] = st
            m8 = _tree(jnp.maximum, st)
            mx[a] = m8 if i == 0 else jnp.maximum(mx[a], m8)
            if i == j:
                mx_s[j, a] = jnp.broadcast_to(jnp.max(mx[a], axis=0, keepdims=True), (8, 128))

    def sm_step(g, j, i, acc):
        for a in range(G):
            h = G * g + a
            base = 64 * (h // HPT) + 8 * (h % HPT)
            st = s_refs[j][a, 128 * i:128 * (i + 1), :]
            m = mx_s[j, a]
            p = jnp.exp2(st.reshape(16, 8, 128) - m[None]).reshape(128, 128).astype(bf16)
            vw = vt_s[base:base + 16, 128 * i:128 * (i + 1)]
            vw = jnp.where(lax.broadcasted_iota(jnp.int32, (16, 128), 0) == 15,
                           jnp.uint32(0x3F803F80), vw)
            d = jnp.dot(_unpack(vw), p, preferred_element_type=f32)
            acc[a] = d if i == 0 else acc[a] + d
            if i == j:
                scale = g1_s[h] / acc[a][24:32]
                ow_s[h, :, 128 * j:128 * (j + 1)] = acc[a] * scale[6:7]

    steps = [(g, j, i) for g in range(H // G) for (j, i) in STEPS]

    def attention():
        qs, mx, acc = [None] * G, [None] * G, [None] * G
        for n, step in enumerate(steps):
            qk_step(*step, qs, mx)
            if n >= LAG:
                sm_step(*steps[n - LAG], acc)

        def tail():
            for step in steps[len(steps) - LAG:]:
                sm_step(*step, acc)
                yield
        return tail()

    def project(t):
        rows = 64 if t < NT - 1 else 40
        w = wc_s[t]
        w = jnp.concatenate([w[0:rows], w[64:64 + rows], w[128:128 + rows]], axis=0)
        qkv = jnp.dot(_unpack(w), _unpack(lnt_s[...]), preferred_element_type=f32)
        n = 2 * rows

        def full(u):
            return u if rows == 64 else jnp.concatenate(
                [u, jnp.zeros((64 - rows, L), u32)], axis=0)

        qf, kf, vf = _eo(qkv[0:n]), _eo(qkv[n:2 * n]), _eo(qkv[2 * n:3 * n])
        q_s[t] = full(_merge(qf[0] * QSCALE, qf[1] * QSCALE))
        k_s[t] = _pack(_unpack(full(_merge(*kf))).T)
        vt = full(_merge(*vf))
        vt_s[64 * t:64 * (t + 1), :] = vt
        pq_s[t] = full(_merge(_phi(qf[0]), _phi(qf[1])))
        pk_s[t] = full(_merge(_phi(kf[0]), _phi(kf[1])))

    def memory_read(t):
        erow = lax.broadcasted_iota(jnp.int32, (128, 128), 0)
        dcol = lax.broadcasted_iota(jnp.int32, (128, 128), 1)
        bd_mask = (erow // DH == dcol // DH) & (dcol < HPT * DH)
        zrow = lax.broadcasted_iota(jnp.int32, (16, 128), 0)
        zcol = lax.broadcasted_iota(jnp.int32, (16, 128), 1)
        z_mask = (zcol // DH == zrow) & (zcol < HPT * DH)
        mt = m_s[t]
        pq = _unpack(pq_s[t])
        mb = jnp.where(bd_mask, mt * gl_s[0:1, 128 * t:128 * (t + 1)], 0.0)
        zb = jnp.where(z_mask, jnp.broadcast_to(mt[126:127, :], (16, 128)), 0.0)
        nd = jnp.dot(jnp.concatenate([mb, zb], axis=0).astype(bf16), pq,
                     preferred_element_type=f32)
        inv = 1.0 / (nd[128:136] + 1e-6)
        row8 = lax.broadcasted_iota(jnp.int32, (8, L), 0)
        bro = [jnp.broadcast_to(inv[a:a + 1], (8, L)) for a in range(HPT)]
        for u in range(16):
            ha, hb = (8 * u) // DH, min((8 * u + 7) // DH, HPT - 1)
            sc = bro[ha] if ha == hb else jnp.where(row8 < DH * hb - 8 * u, bro[ha], bro[hb])
            am_s[128 * t + 8 * u:128 * t + 8 * (u + 1), :] = nd[8 * u:8 * (u + 1)] * sc

    def memory_update(t):
        vone = jnp.where(lax.broadcasted_iota(jnp.int32, (64, L), 0) == 63,
                         jnp.uint32(0x3F803F80), vt_s[64 * t:64 * (t + 1), :])
        m_s[t] += lax.dot_general(_unpack(vone), _unpack(pk_s[t]), NT_DIMS,
                                  preferred_element_type=f32)

    def mix_tile(j):
        cs = slice(128 * j, 128 * (j + 1))
        row8 = lax.broadcasted_iota(jnp.int32, (8, 128), 0)
        parts = []
        for t in range(NT):
            for u in range(16):
                rr, half = u // 2, u % 2
                h = HPT * t + rr
                cut = 2 * rr - 8 * half
                lo_ok, hi_ok = (rr > 0 and h - 1 < H), (rr < HPT and h < H)
                lo = ow_s[h - 1, 16 + 8 * half:24 + 8 * half, cs] if lo_ok else None
                hi = ow_s[h, 8 * half:8 * half + 8, cs] if hi_ok else None
                if cut <= 0 or not lo_ok:
                    dp = hi
                elif cut >= 8 or not hi_ok:
                    dp = lo
                else:
                    dp = jnp.where(row8 >= cut, hi, lo)
                am = am_s[128 * t + 8 * u:128 * t + 8 * (u + 1), cs]
                parts.append(am if dp is None else am + dp)
            ob_tiles[j % 2][64 * t:64 * (t + 1), :] = _merge(
                jnp.concatenate(parts[0::2], axis=0), jnp.concatenate(parts[1::2], axis=0))
            parts = []
            if t % 2 == 1:
                yield
        yield

    def out_proj_tile(s, j):
        cs = slice(128 * j, 128 * (j + 1))
        for c in range(4):
            w = _unpack(wot_s[72 * c:72 * (c + 1), :])
            attn = _eo(jnp.dot(w, _unpack(ob_tiles[j % 2][...]), preferred_element_type=f32))
            x = _split(_pack(xt_s[s, 144 * c:144 * (c + 1), cs]))
            hb = _merge(x[0] + attn[0], x[1] + attn[1])
            h_tiles[j][72 * c:72 * (c + 1), :] = hb
            h_s[4 * s + j, 72 * c:72 * (c + 1), :] = hb
            yield

    def ln2_tile(s, j):
        cs = slice(128 * j, 128 * (j + 1))
        score = []

        def store(lo, hi, h, hn):
            out_s[s, 2 * lo:2 * hi, cs] = _unpack(_merge(h[0] + hn[0], h[1] + hn[1]))
            hn_s[4 * s + j, lo:hi, :] = _merge(*hn)
            score.append(_tree(jnp.add, hn[0] * wr_s[0, lo:hi])
                         + _tree(jnp.add, hn[1] * wr_s[1, lo:hi]))
            if hi == D // 2:
                r_s[s, :, cs] = (score[0] + score[1]) + (score[2] + score[3])
        return ln_steps(lambda lo: h_tiles[j][pl.ds(lo, 72), :], store)

    wq_t = _head_rows(lambda i: _col_block_t(wq_s, i))
    wk_t = _head_rows(lambda i: _col_block_t(wk_s, i))
    wv_t = _head_rows(lambda i: _col_block_t(wv_s, i))
    wo_t = _head_rows(lambda i: _row_block(wo_s, i))

    def first_weights():
        for rows, tiles in ((0, wq_t), (64, wk_t), (128, wv_t)):
            wc_s[0, rows:rows + 64, :] = _eo_rows(next(tiles))
            yield

    def first_ln(j):
        x0_cp[j].wait()
        for c in w_cp[j + 1]:
            c.start()
        yield from ln1_tile(0, j)

    for j in range(4):
        _interleave(first_ln(j))
    def next_weights(t):
        wc_s[t] = jnp.concatenate(
            [_eo_rows(next(wq_t)), _eo_rows(next(wk_t)), _eo_rows(next(wv_t))], axis=0)

    def next_wo(t):
        wot_s[:, 128 * t:128 * (t + 1)] = _eo_rows(_pack(_unpack(_pair_rows(next(wo_t))).T))

    for c in w_cp[0]:
        c.wait()
    wo_cp.start()
    _interleave(first_weights())
    project(0)
    for c in w_cp[1] + w_cp[2]:
        c.wait()
    next_weights(1)
    next_weights(2)
    project(1)
    for c in w_cp[3] + w_cp[4] + [wo_cp]:
        c.wait()
    for c in x_cp[1:] + f_cp:
        c.start()
    for t in (2, 3, 4):
        if t < 4:
            next_weights(t + 1)
        project(t)
        for u in ((0,), (1, 2), (3, 4))[t - 2]:
            next_wo(u)

    def segment(s, last):
        if not last:
            pltpu.make_async_copy(xt_s.at[s + 1], xt_s.at[s + 1], sem_x.at[4 + s]).wait()

        tail = attention()

        def reads():
            for t in range(NT):
                memory_read(t)
                yield

        def updates():
            for t in range(NT):
                memory_update(t)
                yield

        _interleave(reads(), tail)
        _interleave(mix_tile(0), *([] if last else [updates()]))
        for j in range(4):
            gens = [out_proj_tile(s, j)]
            if not last:
                gens.append(ln1_tile(s + 1, j))
            if j < 3:
                gens.append(mix_tile(j + 1))
            if j > 0:
                gens.append(ln2_tile(s, j - 1))
            _interleave(*gens)

        def finish():
            yield from ln2_tile(s, 3)
            lo = s * L if last else pl.multiple_of(s * L, L)
            pltpu.make_async_copy(out_s.at[s], o_hbm.at[:, pl.ds(lo, L)], sem_o.at[s]).start()

        def next_projections():
            for t in range(NT):
                project(t)
                yield

        if last:
            _interleave(finish())
        else:
            _interleave(next_projections(), finish())

    def segment_body(s, carry):
        segment(s, False)
        return carry

    lax.fori_loop(0, NSEG - 1, segment_body, 0)
    segment(NSEG - 1, True)

    rall = jnp.concatenate([_rb(jnp.sum(r_s[s], axis=0, keepdims=True))
                            for s in range(NSEG)], axis=0)
    rmax = jnp.max(rall)
    pos = (lax.broadcasted_iota(jnp.int32, (NSEG, L), 0) * L
           + lax.broadcasted_iota(jnp.int32, (NSEG, L), 1))
    idx = jnp.clip(jnp.min(jnp.where(rall == rmax, pos, S)), 0, S - 1)
    tt = idx // 128
    ln_sel = idx - tt * 128
    rsel = _rb(jax.nn.sigmoid(jnp.full((1, 1), rmax, f32)))
    onehot = (lax.broadcasted_iota(jnp.int32, (16, 128), 1) == ln_sel).astype(bf16)
    xsel = lax.dot_general(onehot, _unpack(hn_s[tt]), NT_DIMS,
                           preferred_element_type=f32).astype(bf16)
    for c in f_cp:
        c.wait()

    def swiglu(c):
        cs = slice(FC * c, FC * (c + 1))
        gate = _rb(jnp.dot(xsel, wg_s[:, cs], preferred_element_type=f32)[0:8])
        up = _rb(jnp.dot(xsel, wu_s[:, cs], preferred_element_type=f32)[0:8])
        return _rb(_rb(gate * jax.nn.sigmoid(gate)) * up)

    def down(c, gu):
        for g in range(D // 16):
            rows = slice(8 * g, 8 * (g + 1))
            acc = [ya_s[k, rows] for k in range(2)] if c > 0 else [None, None]
            for i in range(FC // 128):
                lo = FC * c + 128 * i
                w = _split(_pack(wdt_s[16 * g:16 * (g + 1), lo:lo + 128]))
                for k in range(2):
                    term = w[k] * gu[:, 128 * i:128 * (i + 1)]
                    acc[k] = term if acc[k] is None else acc[k] + term
            for k in range(2):
                ya_s[k, rows] = acc[k]

    gu = swiglu(0)
    for c in range(F // FC):
        nxt = swiglu(c + 1) if c + 1 < F // FC else None
        down(c, gu)
        gu = nxt
    chosen = lax.broadcasted_iota(jnp.int32, (D // 2, 128), 1) == ln_sel
    h_t, hn_t = _split(h_s[tt]), _split(hn_s[tt])
    out = []
    for k in range(2):
        y = _rb(_rb(jnp.sum(ya_s[k], axis=1, keepdims=True)) * rsel)
        out.append(h_t[k] + _rb(hn_t[k] + jnp.where(chosen, y, 0.0)))
    patch_s[...] = _unpack(_merge(*out))
    for s in range(NSEG):
        pltpu.make_async_copy(out_s.at[s], o_hbm.at[:, s * L:(s + 1) * L], sem_o.at[s]).wait()
    cp = pltpu.make_async_copy(patch_s, o_hbm.at[:, pl.ds(pl.multiple_of(tt * 128, 128), 128)],
                               sem_o.at[NSEG])
    cp.start()
    cp.wait()


@jax.jit
def pallas_sequential_preLN__memory_aug_infini_attn__moe_arch_mod__prompt_kernel(
    A_x: jax.Array,
    A_wq: jax.Array,
    A_wk: jax.Array,
    A_wv: jax.Array,
    A_wo: jax.Array,
    A_beta: jax.Array,
    B_x: jax.Array,
    B_w_r: jax.Array,
    B_w_gate: jax.Array,
    B_w_up: jax.Array,
    B_w_down: jax.Array,
):
    del B_x
    vmem = pl.BlockSpec(memory_space=pltpu.VMEM)
    hbm = pl.BlockSpec(memory_space=pltpu.HBM)
    out_t = pl.pallas_call(
        _kernel,
        out_shape=jax.ShapeDtypeStruct((D, S), bf16),
        in_specs=[hbm, hbm, hbm, hbm, hbm, vmem, vmem, hbm, hbm, hbm],
        out_specs=hbm,
        scratch_shapes=[
            pltpu.VMEM((NSEG, D, L), bf16),
            pltpu.VMEM((D, D), bf16),
            pltpu.VMEM((D, D), bf16),
            pltpu.VMEM((D, D), bf16),
            pltpu.VMEM((D, D), bf16),
            pltpu.VMEM((NT, 192, D), u32),
            pltpu.VMEM((D // 2, DP), u32),
            pltpu.VMEM((8, DP), f32),
            pltpu.VMEM((H, 8, 128), f32),
            pltpu.VMEM((2, D // 2, 128), f32),
            pltpu.VMEM((D // 2, L), u32),
            pltpu.VMEM((NT, 64, L), u32),
            pltpu.VMEM((NT, L // 2, 128), u32),
            pltpu.VMEM((DP // 2, L), u32),
            pltpu.VMEM((NT, 64, L), u32),
            pltpu.VMEM((NT, 64, L), u32),
            pltpu.VMEM((DP, L), f32),
            pltpu.VMEM((H, 32, L), f32),
            pltpu.VMEM((G, 128, 128), f32),
            pltpu.VMEM((G, 256, 128), f32),
            pltpu.VMEM((G, 384, 128), f32),
            pltpu.VMEM((G, 512, 128), f32),
            pltpu.VMEM((4, G, 8, 128), f32),
            pltpu.VMEM((NT, 128, 128), f32),
            *[pltpu.VMEM((DP // 2, 128), u32)] * 2,
            *[pltpu.VMEM((D // 2, 128), u32)] * 4,
            pltpu.VMEM((S // 128, D // 2, 128), u32),
            pltpu.VMEM((S // 128, D // 2, 128), u32),
            pltpu.VMEM((NSEG, 8, L), f32),
            pltpu.VMEM((NSEG, D, L), bf16),
            pltpu.VMEM((D, 128), bf16),
            pltpu.VMEM((2, D // 2, 128), f32),
            pltpu.VMEM((D, F), bf16),
            pltpu.VMEM((D, F), bf16),
            pltpu.VMEM((D, F), bf16),
            pltpu.SMEM((4,), jnp.int32),
            pltpu.SemaphoreType.DMA((3 + NSEG,)),
            pltpu.SemaphoreType.DMA((3 * NT + 1,)),
            pltpu.SemaphoreType.DMA((3,)),
            pltpu.SemaphoreType.DMA((NSEG + 1,)),
        ],
        compiler_params=pltpu.CompilerParams(vmem_limit_bytes=100 * 1024 * 1024),
    )(A_x.reshape(S, D).T, A_wq, A_wk, A_wv, A_wo, A_beta, B_w_r,
      B_w_gate, B_w_up, B_w_down.T)
    return out_t.T.reshape(1, S, D)
```
